```python
import os as _os
_os.environ.setdefault("JAX_PLATFORMS", "cpu")
import jax
import jax.numpy as jnp

def _softmax(x, axis=-1):
    return jax.nn.softmax(x, axis=axis)
def _gelu(x):
    return jax.nn.gelu(x, approximate=True)
def _silu(x):
    return jax.nn.silu(x)
def _sigmoid(x):
    return jax.nn.sigmoid(x)
def _layernorm(x, axis=-1, eps=1e-5):
    m = jnp.mean(x, axis=axis, keepdims=True)
    v = jnp.var(x, axis=axis, keepdims=True)
    return (x - m) / jnp.sqrt(v + eps)
def _scatter_add(tgt, idx, src, axis=0):
    return tgt.at[idx].add(src)
def _segment_sum(src, seg, n):
    return jax.ops.segment_sum(src, seg, n)
class _Rng:
    def __init__(self, key):
        self._k = key
    def _next(self):
        self._k, sub = jax.random.split(self._k)
        return sub
    def normal(self, shape):
        return jax.random.normal(self._next(), shape, dtype=jnp.bfloat16)
    def randint(self, lo, hi, shape):
        return jax.random.randint(self._next(), shape, lo, hi, dtype=jnp.int32)
    def uniform(self, shape, lo=0.0, hi=1.0):
        return jax.random.uniform(self._next(), shape, jnp.bfloat16, lo, hi)
    def permutation(self, n):
        return jax.random.permutation(self._next(), n)


kernel_name = 'sequential_preLN__sliding_block__dense_activation_relu__prompt'

def setup_inputs():
    _rng = _Rng(jax.random.key(int.from_bytes(__import__("os").urandom(4), "little")))
    _w = (lambda a: (lambda t: t.astype(jnp.bfloat16) if jnp.issubdtype(t.dtype, jnp.floating) else t)(jnp.asarray(a)))
    def _A_setup():
        B, S, D = 1, 2048, 640
        return {
            "x": _w((lambda *s: _rng.normal(s) * 0.05)(B, S, D)),
            "wqkv": _w((lambda *s: _rng.normal(s) * 0.05)(D, 3 * D)),
            "wo": _w((lambda *s: _rng.normal(s) * 0.05)(D, D)),
        }
    _A_in = _A_setup()

    def _B_setup():
        B, S, D, Dff = 1, 2048, 640, 1536
        return {
            "x": _w((lambda *s: _rng.normal(s) * 0.05)(B, S, D)),
            "w1": _w((lambda *s: _rng.normal(s) * 0.05)(D, Dff)),
            "w2": _w((lambda *s: _rng.normal(s) * 0.05)(Dff, D)),
        }
    _B_in = _B_setup()

    return {
        "A_x": _A_in["x"],
        "A_wqkv": _A_in["wqkv"],
        "A_wo": _A_in["wo"],
        "B_x": _B_in["x"],
        "B_w1": _B_in["w1"],
        "B_w2": _B_in["w2"],
    }

def reference(A_x, A_wqkv, A_wo, B_x, B_w1, B_w2):
    def _A_ref(x, wqkv, wo):
        B, S, D = x.shape
        H = 32; Dh = D // H; W = 256
        qkv = (lambda x, *d: x.transpose(*d))((x @ wqkv).reshape(B, S, 3, H, Dh), 2, 0, 3, 1, 4)
        q, k, v = qkv[0], qkv[1], qkv[2]
        scores = jnp.einsum("bhqd,bhkd->bhqk", q, k) * (Dh ** -0.5)
        idx = jnp.arange(S)
        mask = (idx[:, None] - idx[None, :] >= 0) & (idx[:, None] - idx[None, :] < W)
        scores = jnp.where(mask[None, None], scores, -1e9)
        p = _softmax(scores, axis=-1)
        o = jnp.einsum("bhqk,bhkd->bhqd", p, v)
        return (lambda x, *d: x.transpose(*d))(o, 0, 2, 1, 3).reshape(B, S, D) @ wo

    def _B_ref(x, w1, w2):
        h = jnp.einsum("bsd,df->bsf", x, w1)
        zero = jnp.zeros_like(h)
        h = jnp.maximum(h, zero)
        return jnp.einsum("bsf,fd->bsd", h, w2)

    x = A_x
    h = x + _A_ref(_layernorm(x, axis=-1), A_wqkv, A_wo)
    h2 = h + _B_ref(_layernorm(h, axis=-1), B_w1, B_w2)
    return h2
```

```python
import functools
import math
import jax
import jax.numpy as jnp
from jax import lax
from jax.experimental import pallas as pl
from jax.experimental.pallas import tpu as pltpu

S, D, H, DH, W, DFF = 2048, 640, 32, 20, 256, 1536
TQ = 256
NB = S // TQ
NQB = TQ // 128
NG = 8
GW = 4 * DH
EPS = 1e-5
LOG2E = math.log2(math.e)
QSCALE = DH ** -0.5 * LOG2E
NEG = -1e9 * LOG2E
bf = jnp.bfloat16
f32 = jnp.float32
u32 = jnp.uint32
NT = (((1,), (1,)), ((), ()))
PACKED_D = True
WSPLIT = 256


def _pk(a):
    return pltpu.bitcast(a, u32)


def _up(a):
    return pltpu.bitcast(a, bf)


def _ln(x):
    m = jnp.mean(x, axis=-1, keepdims=True)
    xc = x - m
    v = jnp.mean(xc * xc, axis=-1, keepdims=True)
    return xc * lax.rsqrt(v + EPS)


def _group_chunk(a, g, lane):
    lo = GW * g
    c0, c1 = lo // 128, (lo + GW - 1) // 128
    if c0 == c1:
        return a[:, 128 * c0:128 * c0 + 128]
    return jnp.where(lane >= lo % 128, a[:, 128 * c0:128 * c0 + 128], a[:, 128 * c1:128 * c1 + 128])


def _not_head_lanes(h, lane):
    lo = (DH * h) % 128
    hi = lo + DH
    if hi <= 128:
        return (lane < lo) | (lane >= hi)
    return (lane < lo) & (lane >= hi - 128)


def kernel(x_hbm, wqkv_hbm, wo_hbm, w1_hbm, w2_hbm, o_ref,
           kwin, vwin, wvt, qbuf, obuf, xall, wq_ref, wk_ref, wv_ref, wo_ref, w1_ref, w2_ref, sems, xsems):
    step = pl.program_id(0)
    HW = W // 2
    HT = TQ // 2

    def cp_x(i):
        r = i * TQ if isinstance(i, int) else pl.multiple_of(i * TQ, TQ)
        return pltpu.make_async_copy(x_hbm.at[0, pl.ds(r, TQ), :], xall.at[pl.ds(r, TQ), :], xsems.at[i])

    cp_ka = pltpu.make_async_copy(wqkv_hbm.at[:, D:D + WSPLIT], wk_ref.at[:, 0:WSPLIT], sems.at[0])
    cp_kb = pltpu.make_async_copy(wqkv_hbm.at[:, D + WSPLIT:2 * D], wk_ref.at[:, WSPLIT:D], sems.at[1])
    cp_qa = pltpu.make_async_copy(wqkv_hbm.at[:, 0:WSPLIT], wq_ref.at[:, 0:WSPLIT], sems.at[2])
    cp_qb = pltpu.make_async_copy(wqkv_hbm.at[:, WSPLIT:D], wq_ref.at[:, WSPLIT:D], sems.at[3])
    cp_v = pltpu.make_async_copy(wqkv_hbm.at[:, 2 * D:3 * D], wv_ref, sems.at[4])
    cp_o = pltpu.make_async_copy(wo_hbm, wo_ref, sems.at[5])
    cp_1 = pltpu.make_async_copy(w1_hbm, w1_ref, sems.at[6])
    cp_2 = pltpu.make_async_copy(w2_hbm, w2_ref, sems.at[7])

    def xrows(i):
        r = i * TQ if isinstance(i, int) else pl.multiple_of(i * TQ, TQ)
        return r

    def shift():
        kwin[0:HW, :] = kwin[HT:HT + HW, :]
        vwin[:, 0:W] = vwin[:, TQ:TQ + W]

    def stage_a(blk, r0, R, waits=None):
        HR = R // 2
        h0 = r0 // 2
        lane_h = lax.broadcasted_iota(jnp.int32, (HR, 128), 1)
        st = {}

        def get_xn():
            if 'xn' not in st:
                st['xn'] = _ln(xall[pl.ds(xrows(blk) + r0, R), :].astype(f32)).astype(bf)
            return st['xn']

        def proj(w_ref, wa, wb):
            xn = get_xn()
            if wa is None:
                return jnp.dot(xn, w_ref[...], preferred_element_type=f32)
            wa.wait()
            pa = jnp.dot(xn, w_ref[:, 0:WSPLIT], preferred_element_type=f32)
            wb.wait()
            pb = jnp.dot(xn, w_ref[:, WSPLIT:D], preferred_element_type=f32)
            return jnp.concatenate([pa, pb], axis=1)

        def a_k():
            k = proj(wk_ref, *(waits[0:2] if waits else (None, None)))
            kp = _pk(k.astype(bf))
            for g in range(NG):
                kwin[HW + h0:HW + h0 + HR, 128 * g:128 * g + 128] = _group_chunk(kp, g, lane_h)

        def a_q():
            q = proj(wq_ref, *(waits[2:4] if waits else (None, None))) * QSCALE
            qp = _pk(q.astype(bf))
            for g in range(NG):
                qbuf[h0:h0 + HR, 128 * g:128 * g + 128] = _group_chunk(qp, g, lane_h)

        def a_v():
            vt = lax.dot_general(_up(wvt[...]), get_xn(), NT, preferred_element_type=f32)
            row32 = lax.broadcasted_iota(jnp.int32, (32, R), 0)
            for h in range(H):
                rr = 16 * ((DH * h) // 16)
                jr = 0 if h % 4 == 3 else 31
                win = jnp.where(row32 == jr, 1.0, vt[rr:rr + 32, :])
                vwin[16 * h:16 * h + 16, W + r0:W + r0 + R] = _pk(win.astype(bf))
        return [a_k, a_q, a_v]

    def v3(s):
        return s.reshape(s.shape[0] // 8, 8, 128)

    def local_softmax(s):
        m = jnp.broadcast_to(jnp.max(jnp.max(v3(s), axis=0), axis=0, keepdims=True), (8, 128))
        return jnp.exp2(v3(s) - m[None]).reshape(s.shape), m

    def b_qk(qb, g, nprev):
        lane16 = lax.broadcasted_iota(jnp.int32, (16, 128), 1)
        lane32 = lax.broadcasted_iota(jnp.int32, (32, 128), 1)
        r32 = lax.broadcasted_iota(jnp.int32, (32, 128), 0)
        diag_first = r32 > (lane32 % 32)
        hb = 64 * qb
        cs = slice(128 * g, 128 * g + 128)
        zero16 = jnp.zeros((16, 128), u32)
        nhm = [_not_head_lanes(4 * g + i, lane16) for i in range(4)]
        qs = [qbuf[hb + 16 * j:hb + 16 * j + 16, cs] for j in range(4)]
        M = [[jnp.where(nhm[i], zero16, qs[j]) for j in range(4)] for i in range(4)]
        F = [[None] * 4 for _ in range(4)]
        L = [[None] * 4 for _ in range(4)]
        mD, mW, PW = [], [], []
        cv = (lambda a: _pk(a.astype(bf))) if PACKED_D else (lambda a: a)
        rb = 16 if PACKED_D else 32
        for j in range(4):
            dt = _up(jnp.concatenate([M[(a - j) % 4][j] for a in range(4)], axis=0))
            klast = kwin[hb + 128:hb + 128 + 16 * (j + 1), cs]
            if nprev == 2:
                kk = _up(jnp.concatenate([kwin[hb + 16 * j:hb + 64, cs], klast], axis=0))
                sd = lax.dot_general(kk, dt, NT, preferred_element_type=f32)
                e = jnp.where(diag_first, sd[0:32], sd[128:160])
                sd = jnp.concatenate([e, sd[32:128]], axis=0)
            else:
                sd = lax.dot_general(_up(klast), dt, NT, preferred_element_type=f32)
                e = jnp.where(diag_first, NEG, sd[32 * j:32 * j + 32])
                sd = jnp.concatenate([e, sd[0:32 * j]], axis=0) if j else e
            pd, m = local_softmax(sd)
            mD.append(m)
            e = pd[0:32]
            rest = cv(pd[32:]) if pd.shape[0] > 32 else None
            n = 0
            if nprev == 2:
                F[j][j] = cv(jnp.where(diag_first, e, 0.0))
                L[j][j] = cv(jnp.where(diag_first, 0.0, e))
                for b in range(j + 1, 4):
                    F[b][j] = rest[rb * n:rb * n + rb]; n += 1
            else:
                L[j][j] = cv(e)
            for b in range(0, j):
                L[b][j] = rest[rb * n:rb * n + rb]; n += 1
        if nprev >= 1:
            kmid = _up(kwin[hb + 64:hb + 128, cs])
            for i in range(4):
                wt = _up(jnp.concatenate([M[i][(a - i) % 4] for a in range(4)], axis=0))
                pw, m = local_softmax(lax.dot_general(kmid, wt, NT, preferred_element_type=f32))
                PW.append(pw.astype(bf))
                mW.append(m)
        return F, L, mD, PW, mW

    def exchange(src, lane):
        grp = lane // 32
        odd = (grp & 1) == 1
        hi = grp >= 2
        live = [j for j in range(4) if src[j] is not None]

        def sel(m, a, b):
            if a is None:
                return b
            if b is None:
                return a
            return jnp.where(m, a, b)
        if len(live) == 2:
            out = []
            for i in range(4):
                ga = [(j + i) % 4 for j in live]
                m = (grp == ga[0])
                out.append(jnp.where(m, src[live[0]], src[live[1]]))
        else:
            t = [sel(odd, src[(j + 1) % 4], src[j]) for j in range(4)]
            out = [sel(hi, t[(2 - i) % 4], t[(-i) % 4]) for i in range(4)]
        if len(live) < 4:
            res = []
            for i in range(4):
                dead = [(j + i) % 4 for j in range(4) if j not in live]
                m = grp == dead[0]
                for dd in dead[1:]:
                    m = m | (grp == dd)
                res.append(jnp.where(m, jnp.zeros_like(out[i]), out[i]))
            out = res
        return out

    def b_pv(qb, g, nprev, F, L, mD, PW, mW):
        laneP = lax.broadcasted_iota(jnp.int32, (16 if PACKED_D else 32, 128), 1)
        lane8 = lax.broadcasted_iota(jnp.int32, (8, 128), 1)
        sub8 = lax.broadcasted_iota(jnp.int32, (8, 128), 0)
        base = 128 * qb
        fin = _up if PACKED_D else (lambda a: a.astype(bf))
        Fx = [exchange(F[b], laneP) for b in range(4)] if nprev == 2 else None
        Lx = [exchange(L[b], laneP) for b in range(4)]
        if nprev >= 1:
            mE = exchange(mD, lane8)
        os_ = []
        for i in range(4):
            h = 4 * g + i
            rows = slice(16 * h, 16 * h + 16)
            vl = vwin[rows, base + 256:base + 384]
            if nprev == 2:
                pe = fin(jnp.concatenate([Fx[b][i] for b in range(4)] + [Lx[b][i] for b in range(4)], axis=0))
                ve = _up(jnp.concatenate([vwin[rows, base:base + 128], vl], axis=1))
            else:
                pe = fin(jnp.concatenate([Lx[b][i] for b in range(4)], axis=0))
                ve = _up(vl)
            res = jnp.dot(ve, pe, preferred_element_type=f32)
            if nprev >= 1:
                resm = jnp.dot(_up(vwin[rows, base + 128:base + 256]), PW[i], preferred_element_type=f32)
                mx = jnp.maximum(mE[i], mW[i])
                ae = jnp.exp2(mE[i] - mx)
                am = jnp.exp2(mW[i] - mx)
                res = (v3(res) * ae[None] + v3(resm) * am[None]).reshape(32, 128)
            jr = 0 if i == 3 else 31
            inv = 1.0 / res[jr:jr + 1, :]
            lo = (0, 0, 8, 8)[i]
            o = res[lo:lo + 24] * inv
            if i:
                o = pltpu.roll(o, 128 - 32 * i, 1)
            os_.append(o)
        o0, o1, o2, o3 = os_
        return [o0[0:16], jnp.where(sub8 < 4, o0[16:24], o1[0:8]), o1[8:24],
                o2[0:16], jnp.where(sub8 < 4, o2[16:24], o3[0:8]), o3[8:24]]

    def b_fin(qb, parts):
        ot = jnp.concatenate(parts, axis=0)
        obuf[64 * qb:64 * qb + 64, :] = _pk(ot.astype(bf).T)

    def run_attention(fillers, first_step, sched, order='A'):
        items = [(qb, g, min(qb, 2) if first_step else 2) for qb in range(NQB) for g in range(NG)]
        pend = []
        issued = 0
        parts = []
        for n, (qb, g, nprev) in enumerate(items):
            if order == 'B':
                if issued == 0:
                    pend.append(b_qk(*items[0])); issued = 1
                for f in fillers.get(n, []):
                    f()
            while issued < min(sched(n), len(items)):
                pend.append(b_qk(*items[issued]))
                issued += 1
            if order != 'B':
                for f in fillers.get(n, []):
                    f()
            parts += b_pv(qb, g, nprev, *pend.pop(0))
            if g == NG - 1:
                b_fin(qb, parts)
                parts = []
        for f in fillers.get(len(items), []):
            f()

    def stage_c(blk, nsplit):
        R = TQ // nsplit
        res = []
        for sp in range(nsplit):
            st = {}
            r0 = sp * R

            def c_wo(st=st, r0=r0):
                hres = xall[pl.ds(xrows(blk) + r0, R), :].astype(f32) + jnp.dot(
                    _up(obuf[r0 // 2:(r0 + R) // 2, :]), wo_ref[...], preferred_element_type=f32)
                st['h'] = hres
                st['hn'] = _ln(hres).astype(bf)
                st['f1'] = []
                st['f1b'] = {}
                st['acc'] = {}

            def c_f1(c, st=st):
                def f():
                    v = jnp.dot(st['hn'], w1_ref[:, 256 * c:256 * c + 256], preferred_element_type=f32)
                    st['f1'].append(jnp.maximum(v, 0.0))
                return f

            def c_f2(c, kh, st=st, r0=r0):
                def f():
                    if kh not in st['f1b']:
                        st['f1b'][kh] = jnp.concatenate(st['f1'][3 * kh:3 * kh + 3], axis=1).astype(bf)
                    v = jnp.dot(st['f1b'][kh], w2_ref[768 * kh:768 * kh + 768, 128 * c:128 * c + 128],
                                preferred_element_type=f32)
                    if kh == 0:
                        st['acc'][c] = st['h'][:, 128 * c:128 * c + 128] + v
                    else:
                        o_ref[0, r0:r0 + R, 128 * c:128 * c + 128] = (st['acc'][c] + v).astype(o_ref.dtype)
                return f
            res.append((c_wo, [c_f1(c) for c in range(6)],
                        [c_f2(c, kh) for kh in range(2) for c in range(5)]))
        return res

    @pl.when(step == 0)
    def _first():
        cp_x(0).start()
        for c in (cp_ka, cp_kb, cp_qa, cp_qb, cp_v, cp_o):
            c.start()
        cp_x(1).start()
        cp_1.start(); cp_2.start()
        for i in range(2, NB):
            cp_x(i).start()
        cp_x(0).wait()
        a_k, a_q, a_v = stage_a(0, 0, TQ, [cp_ka, cp_kb, cp_qa, cp_qb])
        a_k()
        a_q()
        cp_v.wait()
        wvt[...] = _pk(wv_ref[...].T)
        run_attention({0: [a_v]}, True, lambda n: 8 if n < 6 else n + 3)
        cp_o.wait()

    def mid(blk, first):
        cp_x(blk).wait()
        (c_wo, f1s, f2s), = stage_c(blk - 1, 1)
        k0, q0, v0 = stage_a(blk, 0, 128)
        k1, q1, v1 = stage_a(blk, 128, 128)
        shift()
        c_wo()
        k0(); q0()

        def w12():
            cp_1.wait(); cp_2.wait()
        if first:
            order = [[v0], [k1], [q1], [v1], [w12, f1s[0]], [f1s[1]], [f1s[2]], [f1s[3]], [f1s[4]], [f1s[5]],
                     f2s[0:1], f2s[1:2], f2s[2:3], f2s[3:4], f2s[4:6], f2s[6:8], f2s[8:10]]
        else:
            order = [[v0], [f1s[0]], [k1], [f1s[1]], [q1], [f1s[2]], [v1], [f1s[3]], [f1s[4]], [f1s[5]],
                     f2s[0:1], f2s[1:2], f2s[2:3], f2s[3:4], f2s[4:6], f2s[6:8], f2s[8:10]]
        fill = dict(enumerate(order))
        run_attention(fill, False, lambda n: n + 1, 'A')

    @pl.when(step == 1)
    def _second():
        mid(1, True)

    @pl.when(jnp.logical_and(step > 1, step < NB))
    def _mid():
        mid(step, False)

    @pl.when(step == NB)
    def _last():
        (wo0, f10, f20), (wo1, f11, f21) = stage_c(NB - 1, 2)
        wo0(); wo1()
        for f in f10 + f11 + f20 + f21:
            f()


@jax.jit
def pallas_sequential_preLN__sliding_block__dense_activation_relu__prompt_kernel(A_x, A_wqkv, A_wo, B_x, B_w1, B_w2):
    anyspec = pl.BlockSpec(memory_space=pl.ANY)
    return pl.pallas_call(
        kernel,
        grid=(NB + 1,),
        in_specs=[anyspec] * 5,
        out_specs=pl.BlockSpec((1, TQ, D), lambda i: (0, jnp.maximum(i - 1, 0), 0)),
        out_shape=jax.ShapeDtypeStruct((1, S, D), bf),
        scratch_shapes=[
            pltpu.VMEM(((W + TQ) // 2, NG * 128), u32),
            pltpu.VMEM((H * 16, W + TQ), u32),
            pltpu.VMEM((D // 2, D), u32),
            pltpu.VMEM((TQ // 2, NG * 128), u32),
            pltpu.VMEM((TQ // 2, D), u32),
            pltpu.VMEM((S, D), bf),
            pltpu.VMEM((D, D), bf),
            pltpu.VMEM((D, D), bf),
            pltpu.VMEM((D, D), bf),
            pltpu.VMEM((D, D), bf),
            pltpu.VMEM((D, DFF), bf),
            pltpu.VMEM((DFF, D), bf),
            pltpu.SemaphoreType.DMA((8,)),
            pltpu.SemaphoreType.DMA((NB,)),
        ],
        compiler_params=pltpu.CompilerParams(dimension_semantics=("arbitrary",),
                                             vmem_limit_bytes=64 * 1024 * 1024),
        name="fused",
    )(A_x, A_wqkv, A_wo, B_w1, B_w2)
```

```python
import math

import jax
import jax.numpy as jnp
from jax import lax
from jax.experimental import pallas as pl
from jax.experimental.pallas import tpu as pltpu

S, D, H, DH, W, DFF = 2048, 640, 32, 20, 256, 1536
TQ = 256
NB = S // TQ
NG = 8
GW = 4 * DH
EPS = 1e-5
LOG2E = math.log2(math.e)
QSCALE = DH ** -0.5 * LOG2E
NEG = -1e9 * LOG2E
bf = jnp.bfloat16
f32 = jnp.float32
u32 = jnp.uint32
NT = (((1,), (1,)), ((), ()))


def _pk(a):
    return pltpu.bitcast(a, u32)


def _up(a):
    return pltpu.bitcast(a, bf)


def _ln(x):
    m = jnp.mean(x, axis=-1, keepdims=True)
    xc = x - m
    v = jnp.mean(xc * xc, axis=-1, keepdims=True)
    return xc * lax.rsqrt(v + EPS)


def _lane(rows):
    return lax.broadcasted_iota(jnp.int32, (rows, 128), 1)


def _group_cols(g):
    lo = GW * g
    return lo // 128, (lo + GW - 1) // 128


def _not_head_lanes(h, lane):
    lo = (DH * h) % 128
    hi = lo + DH
    if hi <= 128:
        return (lane < lo) | (lane >= hi)
    return (lane < lo) & (lane >= hi - 128)


def _v3(s):
    return s.reshape(s.shape[0] // 8, 8, 128)


def _local_softmax(s):
    m = jnp.broadcast_to(jnp.max(jnp.max(_v3(s), axis=0), axis=0, keepdims=True), (8, 128))
    return jnp.exp2(_v3(s) - m[None]).reshape(s.shape), m


def _exchange(src, lane):
    grp = lane // 32
    odd = (grp & 1) == 1
    hi = grp >= 2
    live = [j for j in range(4) if src[j] is not None]

    def sel(m, a, b):
        if a is None:
            return b
        if b is None:
            return a
        return jnp.where(m, a, b)
    if len(live) == 2:
        out = [jnp.where(grp == (live[0] + i) % 4, src[live[0]], src[live[1]]) for i in range(4)]
    else:
        t = [sel(odd, src[(j + 1) % 4], src[j]) for j in range(4)]
        out = [sel(hi, t[(2 - i) % 4], t[(-i) % 4]) for i in range(4)]
    if len(live) < 4:
        res = []
        for i in range(4):
            dead = [(j + i) % 4 for j in range(4) if j not in live]
            m = grp == dead[0]
            for dd in dead[1:]:
                m = m | (grp == dd)
            res.append(jnp.where(m, jnp.zeros_like(out[i]), out[i]))
        out = res
    return out


def _qk(n, t=''):
    return [('qd' + t, n), ('qw' + t, n)]


def _pv(n, t=''):
    return [('pe' + t, n), ('pm' + t, n)]


def _weave(first, fills):
    prog = []
    for n in range(first, 16):
        prog += fills[n - first] + (_qk(n + 1) if n < 15 else []) + _pv(n)
    return prog


def _kernel(x_hbm, wqkv_hbm, wo_hbm, w1_hbm, w2_hbm, o_hbm,
            kwin, vwin, wvt, qbuf, obuf, xall, oall, wqk_ref, wv_ref, wo_ref, w1_ref, w2_ref, sems):
    step = pl.program_id(0)

    def xrows(i):
        return i * TQ if isinstance(i, int) else pl.multiple_of(i * TQ, TQ)

    def out_start(r, n, c0, c1):
        cols = slice(128 * c0, 128 * c1)
        pltpu.make_async_copy(oall.at[pl.ds(r, n), cols], o_hbm.at[0, pl.ds(r, n), cols], sems.at[12]).start()

    def shift():
        kwin[0:W // 2, :] = kwin[TQ // 2:TQ // 2 + W // 2, :]
        vwin[:, 0:W] = vwin[:, TQ:TQ + W]

    def stage_a(ops, tag, blk, r0, koff=W):
        R = 128
        h0 = r0 // 2
        lane_h = _lane(R // 2)
        st = {'k': {}, 'q': {}, 'kd': set(), 'qd': set()}

        def get_ln():
            if 'ln' not in st:
                st['ln'] = _ln(xall[pl.ds(xrows(blk) + r0, R), :].astype(f32))
            return st['ln']

        def get_xn():
            if 'xn' not in st:
                st['xn'] = get_ln().astype(bf)
            return st['xn']

        def finish(which, c0, c1, p):
            dst, roff = (kwin, koff // 2) if which == 'k' else (qbuf, 0)
            if which == 'q':
                p = p * QSCALE
            p = _pk(p.astype(bf))
            have = st[which]
            for c in range(c0, c1):
                have[c] = p[:, 128 * (c - c0):128 * (c - c0) + 128]
            for g in range(NG):
                a, b = _group_cols(g)
                if g not in st[which + 'd'] and a in have and b in have:
                    st[which + 'd'].add(g)
                    val = have[a] if a == b else jnp.where(lane_h >= (GW * g) % 128, have[a], have[b])
                    dst[roff + h0:roff + h0 + R // 2, 128 * g:128 * g + 128] = val

        def proj(which, c0, c1):
            off = D if which == 'k' else 0
            finish(which, c0, c1, jnp.dot(get_xn(), wqk_ref[:, off + 128 * c0:off + 128 * c1],
                                          preferred_element_type=f32))

        def projk(k):
            p = jnp.dot(get_ln()[:, 128 * k:128 * k + 128].astype(bf), wqk_ref[128 * k:128 * k + 128, :],
                        preferred_element_type=f32)
            if k:
                p = p + st['acc']
            st['acc'] = p
            if k == 4:
                finish('k', 0, 5, p[:, D:2 * D])
                finish('q', 0, 5, p[:, 0:D])

        def vproj(g0, g1):
            vt = lax.dot_general(_up(wvt[40 * g0:40 * g1, :]), get_xn(), NT, preferred_element_type=f32)
            row32 = lax.broadcasted_iota(jnp.int32, (32, R), 0)
            for h in range(4 * g0, 4 * g1):
                rr = 16 * ((DH * h) // 16) - 80 * g0
                jr = 0 if h % 4 == 3 else 31
                win = jnp.where(row32 == jr, 1.0, vt[rr:rr + 32, :])
                vwin[16 * h:16 * h + 16, koff + r0:koff + r0 + R] = _pk(win.astype(bf))
        ops['k' + tag] = lambda c0, c1: proj('k', c0, c1)
        ops['q' + tag] = lambda c0, c1: proj('q', c0, c1)
        ops['v' + tag] = vproj
        ops['ln' + tag] = get_ln
        ops['qk' + tag] = projk

    def stage_b(ops, first_block, tag=''):
        wb = -W if first_block else 0
        items = [(qb, g, min(qb, 2) if first_block else 2) for qb in range(2) for g in range(NG)]
        sts = [dict() for _ in items]
        parts = {0: {}, 1: {}}

        def qmask(n):
            qb, g, _ = items[n]
            st = sts[n]
            if 'M' not in st:
                lane16 = _lane(16)
                zero16 = jnp.zeros((16, 128), u32)
                nhm = [_not_head_lanes(4 * g + i, lane16) for i in range(4)]
                qs = [qbuf[64 * qb + 16 * j:64 * qb + 16 * j + 16, 128 * g:128 * g + 128] for j in range(4)]
                st['M'] = [[jnp.where(nhm[i], zero16, qs[j]) for j in range(4)] for i in range(4)]
            return st['M']

        def qd(n):
            qb, g, nprev = items[n]
            M = qmask(n)
            diag_first = lax.broadcasted_iota(jnp.int32, (32, 128), 0) > (_lane(32) % 32)
            hb = 64 * qb + wb // 2
            cs = slice(128 * g, 128 * g + 128)
            F = [[None] * 4 for _ in range(4)]
            L = [[None] * 4 for _ in range(4)]
            mD = []

            def cv(a):
                return _pk(a.astype(bf))
            for j in range(4):
                dt = _up(jnp.concatenate([M[(a - j) % 4][j] for a in range(4)], axis=0))
                klast = kwin[hb + 128:hb + 128 + 16 * (j + 1), cs]
                if nprev == 2:
                    kk = _up(jnp.concatenate([kwin[hb + 16 * j:hb + 64, cs], klast], axis=0))
                    sd = lax.dot_general(kk, dt, NT, preferred_element_type=f32)
                    e = jnp.where(diag_first, sd[0:32], sd[128:160])
                    sd = jnp.concatenate([e, sd[32:128]], axis=0)
                else:
                    sd = lax.dot_general(_up(klast), dt, NT, preferred_element_type=f32)
                    e = jnp.where(diag_first, NEG, sd[32 * j:32 * j + 32])
                    sd = jnp.concatenate([e, sd[0:32 * j]], axis=0) if j else e
                pd, m = _local_softmax(sd)
                mD.append(m)
                e = pd[0:32]
                rest = cv(pd[32:]) if pd.shape[0] > 32 else None
                k = 0
                if nprev == 2:
                    F[j][j] = cv(jnp.where(diag_first, e, 0.0))
                    L[j][j] = cv(jnp.where(diag_first, 0.0, e))
                    for b in range(j + 1, 4):
                        F[b][j] = rest[16 * k:16 * k + 16]
                        k += 1
                else:
                    L[j][j] = cv(e)
                for b in range(0, j):
                    L[b][j] = rest[16 * k:16 * k + 16]
                    k += 1
            sts[n].update(F=F, L=L, mD=mD)

        def qw(n):
            qb, g, nprev = items[n]
            if nprev == 0:
                return
            st = sts[n]
            M = qmask(n)
            kmid = _up(kwin[wb // 2 + 64 * qb + 64:wb // 2 + 64 * qb + 128, 128 * g:128 * g + 128])
            st['PW'], st['mW'] = [], []
            for i in range(4):
                wt = _up(jnp.concatenate([M[i][(a - i) % 4] for a in range(4)], axis=0))
                pw, m = _local_softmax(lax.dot_general(kmid, wt, NT, preferred_element_type=f32))
                st['PW'].append(pw.astype(bf))
                st['mW'].append(m)

        def pe(n):
            qb, g, nprev = items[n]
            st = sts[n]
            base = 128 * qb + wb
            lane16 = _lane(16)
            Fx = [_exchange(st['F'][b], lane16) for b in range(4)] if nprev == 2 else None
            Lx = [_exchange(st['L'][b], lane16) for b in range(4)]
            st['resE'] = []
            for i in range(4):
                rows = slice(16 * (4 * g + i), 16 * (4 * g + i) + 16)
                vl = vwin[rows, base + 256:base + 384]
                if nprev == 2:
                    p = jnp.concatenate([Fx[b][i] for b in range(4)] + [Lx[b][i] for b in range(4)], axis=0)
                    v = jnp.concatenate([vwin[rows, base:base + 128], vl], axis=1)
                else:
                    p = jnp.concatenate([Lx[b][i] for b in range(4)], axis=0)
                    v = vl
                st['resE'].append(jnp.dot(_up(v), _up(p), preferred_element_type=f32))

        def pm(n):
            qb, g, nprev = items[n]
            st = sts[n]
            base = 128 * qb + wb
            sub8 = lax.broadcasted_iota(jnp.int32, (8, 128), 0)
            if nprev >= 1:
                mE = _exchange(st['mD'], _lane(8))
            os_ = []
            for i in range(4):
                rows = slice(16 * (4 * g + i), 16 * (4 * g + i) + 16)
                res = st['resE'][i]
                if nprev >= 1:
                    resm = jnp.dot(_up(vwin[rows, base + 128:base + 256]), st['PW'][i],
                                   preferred_element_type=f32)
                    mx = jnp.maximum(mE[i], st['mW'][i])
                    ae = jnp.exp2(mE[i] - mx)
                    am = jnp.exp2(st['mW'][i] - mx)
                    res = (_v3(res) * ae[None] + _v3(resm) * am[None]).reshape(32, 128)
                jr = 0 if i == 3 else 31
                inv = 1.0 / res[jr:jr + 1, :]
                lo = (0, 0, 8, 8)[i]
                o = res[lo:lo + 24] * inv
                if i:
                    o = pltpu.roll(o, 128 - 32 * i, 1)
                os_.append(o)
            o0, o1, o2, o3 = os_
            parts[qb][g] = [o0[0:16], jnp.where(sub8 < 4, o0[16:24], o1[0:8]), o1[8:24],
                            o2[0:16], jnp.where(sub8 < 4, o2[16:24], o3[0:8]), o3[8:24]]
            st.clear()
            if len(parts[qb]) == NG:
                ot = jnp.concatenate([p for gg in range(NG) for p in parts[qb][gg]], axis=0)
                obuf[64 * qb:64 * qb + 64, :] = _pk(ot.astype(bf).T)
        ops.update({'qd' + tag: qd, 'qw' + tag: qw, 'pe' + tag: pe, 'pm' + tag: pm})

    def stage_c(ops, tag, blk, r0, R):
        st = {'f1': {}, 'f1b': {}, 'acc': {}}

        def c_wo():
            hres = xall[pl.ds(xrows(blk) + r0, R), :].astype(f32) + jnp.dot(
                _up(obuf[r0 // 2:(r0 + R) // 2, :]), wo_ref[...], preferred_element_type=f32)
            st['h'] = hres
            st['hn'] = _ln(hres).astype(bf)

        def c_f1(c0, c1):
            v = jnp.dot(st['hn'], w1_ref[:, 128 * c0:128 * c1], preferred_element_type=f32)
            v = jnp.maximum(v, 0.0)
            for c in range(c0, c1):
                st['f1'][c] = v[:, 128 * (c - c0):128 * (c - c0) + 128]

        def c_f2(c, k0, k1, ra=0, rb=R):
            key = (k0, k1, ra, rb)
            if key not in st['f1b']:
                st['f1b'][key] = jnp.concatenate(
                    [st['f1'][k][ra:rb] for k in range(k0, k1)], axis=1).astype(bf)
            v = jnp.dot(st['f1b'][key], w2_ref[128 * k0:128 * k1, 128 * c:128 * c + 128],
                        preferred_element_type=f32)
            if k0 == 0:
                acc = st['h'][ra:rb, 128 * c:128 * c + 128] + v
            else:
                acc = st['acc'][c][ra:rb] + v
            if k1 == 12:
                oall[pl.ds(xrows(blk) + r0 + ra, rb - ra), 128 * c:128 * c + 128] = acc.astype(bf)
            else:
                st['acc'][c] = acc
        ops['wo' + tag] = c_wo
        ops['f1' + tag] = c_f1
        ops['f2' + tag] = c_f2
        ops['out' + tag] = lambda c0, c1: out_start(xrows(blk) + r0, R, c0, c1)

    def run(ops, prog):
        for item in prog:
            ops[item[0]](*item[1:])

    @pl.when(step == 0)
    def _first():
        def cp_x(i, r0, r1):
            return pltpu.make_async_copy(x_hbm.at[0, r0:r1, :], xall.at[r0:r1, :], sems.at[i])
        cx0, cx1, cx2 = cp_x(0, 0, TQ), cp_x(1, TQ, 2 * TQ), cp_x(2, 2 * TQ, S)
        cp_qk = [pltpu.make_async_copy(wqkv_hbm.at[128 * k:128 * k + 128, 0:2 * D],
                                       wqk_ref.at[128 * k:128 * k + 128, :], sems.at[3 + k])
                 for k in range(5)]
        cp_v = pltpu.make_async_copy(wqkv_hbm.at[:, 2 * D:3 * D], wv_ref, sems.at[8])
        cp_o = pltpu.make_async_copy(wo_hbm, wo_ref, sems.at[9])
        cp_1 = pltpu.make_async_copy(w1_hbm, w1_ref, sems.at[10])
        cp_2 = pltpu.make_async_copy(w2_hbm, w2_ref, sems.at[11])
        for c in [cx0] + cp_qk + [cx1, cp_v, cp_o, cp_1, cp_2, cx2]:
            c.start()

        ops = {}
        stage_a(ops, 'L', 0, 0, 0)
        stage_a(ops, 'H', 0, 128, 0)
        stage_b(ops, True, 'a')
        stage_a(ops, '0', 1, 0)
        stage_a(ops, '1', 1, 128)
        stage_b(ops, False)
        stage_c(ops, '', 0, 0, TQ)

        def waits(*cps):
            for c in cps:
                c.wait()

        def xpose_wv():
            wvt[...] = _pk(wv_ref[...].T)
        ops.update(wait=waits, xpose=xpose_wv, shift=shift)

        def qa(*ns):
            return [o for n in ns for o in _qk(n, 'a')]

        def pa(*ns):
            return [o for n in ns for o in _pv(n, 'a')]
        prog = [('wait', cx0), ('lnL',), ('lnH',)]
        for k in range(5):
            prog += [('wait', cp_qk[k]), ('qkL', k), ('qkH', k)]
        prog += qa(*range(11))
        prog += [('wait', cx1, cp_v), ('xpose',)]
        prog += qa(11, 12, 13, 14) + [('k0', 0, 2), ('k0', 2, 5)] + qa(15) + [('vL', 0, 4), ('vL', 4, 8)]
        prog += pa(0) + [('q0', 0, 3)] + pa(1, 2) + [('q0', 3, 5)] + pa(3) + [('vH', 0, 8)] + pa(4, 5)
        prog += [('v0', 0, 4)] + _qk(0) + [('v0', 4, 8)] + _qk(1) + _pv(0) + pa(6) + _qk(2) + _pv(1)
        prog += _qk(3) + pa(7, 8) + _pv(2) + [('k1', 0, 2)] + _pv(3) + pa(9, 10) + _qk(4)
        prog += [('k1', 2, 5)] + pa(11, 12, 13, 14, 15) + [('q1', 0, 5)]
        prog += [('wait', cp_o, cp_1, cp_2), ('wo',), ('v1', 0, 4), ('v1', 4, 8)]
        prog += _qk(5) + _pv(4) + _qk(6) + _pv(5)
        prog += _weave(6, [
            [('f1', 0, 2)], [('f1', 2, 4), ('f2', 0, 0, 4)], [('f1', 4, 6)], [('f1', 6, 8)],
            [('f2', 1, 0, 4), ('f1', 8, 10)], [('f1', 10, 12)],
            [('f2', 2, 0, 4), ('f2', 3, 0, 4), ('f2', 4, 0, 4)], [('f2', 0, 4, 8), ('f2', 1, 4, 8)],
            [('f2', 2, 4, 8), ('f2', 3, 4, 8), ('f2', 4, 4, 8)],
            [('f2', 0, 8, 12), ('f2', 1, 8, 12), ('f2', 2, 8, 12)]])
        prog += [('f2', 3, 8, 12), ('shift',), ('f2', 4, 8, 12, 0, 128), ('f2', 4, 8, 12, 128, 256)]
        prog += [('out', 0, 5), ('wait', cx2)]
        run(ops, prog)

    @pl.when(jnp.logical_and(step > 0, step < NB - 1))
    def _mid():
        blk = step + 1
        ops = {'shift': shift}
        stage_c(ops, '', blk - 1, 0, TQ)
        stage_a(ops, '0', blk, 0)
        stage_a(ops, '1', blk, 128)
        stage_b(ops, False)
        prog = [('wo',), ('q0', 0, 5), ('k0', 0, 5)] + _qk(0)
        prog += _weave(0, [
            [('v0', 0, 8)], [('k1', 0, 1), ('f1', 0, 2)], [('k1', 1, 5)], [('q1', 0, 5)], [],
            [('f1', 2, 4)], [('v1', 0, 8)], [('f1', 4, 6)], [('f1', 6, 8)],
            [('f2', 0, 0, 6), ('f1', 8, 9)], [('f1', 9, 10), ('f1', 10, 11)], [('f2', 1, 0, 6)],
            [('f1', 11, 12), ('f2', 2, 0, 6)], [('f2', 3, 0, 6), ('f2', 4, 0, 6)], [('f2', 0, 6, 12)],
            [('f2', 1, 6, 12), ('f2', 2, 6, 12)]])
        prog += [('shift',), ('f2', 3, 6, 12), ('f2', 4, 6, 12, 0, 128), ('f2', 4, 6, 12, 128, 256)]
        prog += [('out', 0, 5)]
        run(ops, prog)

    @pl.when(step == NB - 1)
    def _last():
        ops = {}
        stage_c(ops, '0', NB - 1, 0, 128)
        stage_c(ops, '1', NB - 1, 128, 128)
        prog = [('wo0',), ('wo1',)]
        for t in '01':
            prog += [('f1' + t, 2 * c, 2 * c + 2) for c in range(6)]
        prog += [('f20', c, 0, 12) for c in range(5)] + [('out0', 0, 5)]
        prog += [('f21', c, 0, 12) for c in range(4)] + [('out1', 0, 4), ('f21', 4, 0, 12), ('out1', 4, 5)]
        run(ops, prog)
        pltpu.make_async_copy(oall, o_hbm.at[0], sems.at[12]).wait()


@jax.jit
def pallas_sequential_preLN__sliding_block__dense_activation_relu__prompt_kernel(
    A_x: jax.Array,
    A_wqkv: jax.Array,
    A_wo: jax.Array,
    B_x: jax.Array,
    B_w1: jax.Array,
    B_w2: jax.Array,
):
    del B_x
    hbm = pl.BlockSpec(memory_space=pl.ANY)
    return pl.pallas_call(
        _kernel,
        grid=(NB,),
        in_specs=[hbm] * 5,
        out_specs=hbm,
        out_shape=jax.ShapeDtypeStruct((1, S, D), bf),
        scratch_shapes=[
            pltpu.VMEM(((W + TQ) // 2, NG * 128), u32),
            pltpu.VMEM((H * 16, W + TQ), u32),
            pltpu.VMEM((D // 2, D), u32),
            pltpu.VMEM((TQ // 2, NG * 128), u32),
            pltpu.VMEM((TQ // 2, D), u32),
            pltpu.VMEM((S, D), bf),
            pltpu.VMEM((S, D), bf),
            pltpu.VMEM((D, 2 * D), bf),
            pltpu.VMEM((D, D), bf),
            pltpu.VMEM((D, D), bf),
            pltpu.VMEM((D, DFF), bf),
            pltpu.VMEM((DFF, D), bf),
            pltpu.SemaphoreType.DMA((13,)),
        ],
        compiler_params=pltpu.CompilerParams(
            dimension_semantics=("arbitrary",),
            vmem_limit_bytes=64 * 1024 * 1024,
            disable_bounds_checks=True,
            disable_semaphore_checks=True,
        ),
        name="fused",
    )(A_x, A_wqkv, A_wo, B_w1, B_w2)
```

```python
import math

import jax
import jax.numpy as jnp
from jax import lax
from jax.experimental import pallas as pl
from jax.experimental.pallas import tpu as pltpu

S, D, H, DH, W, DFF = 2048, 640, 32, 20, 256, 1536
TQ = 256
NB = S // TQ
NG = 8
GW = 4 * DH
EPS = 1e-5
LOG2E = math.log2(math.e)
QSCALE = DH ** -0.5 * LOG2E
NEG = -1e9 * LOG2E
bf = jnp.bfloat16
f32 = jnp.float32
u32 = jnp.uint32
NT = (((1,), (1,)), ((), ()))


def _pk(a):
    return pltpu.bitcast(a, u32)


def _up(a):
    return pltpu.bitcast(a, bf)


def _ln(x):
    m = jnp.mean(x, axis=-1, keepdims=True)
    xc = x - m
    v = jnp.mean(xc * xc, axis=-1, keepdims=True)
    return xc * lax.rsqrt(v + EPS)


def _lane(rows):
    return lax.broadcasted_iota(jnp.int32, (rows, 128), 1)


def _group_cols(g):
    lo = GW * g
    return lo // 128, (lo + GW - 1) // 128


def _not_head_lanes(h, lane):
    lo = (DH * h) % 128
    hi = lo + DH
    if hi <= 128:
        return (lane < lo) | (lane >= hi)
    return (lane < lo) & (lane >= hi - 128)


def _v3(s):
    return s.reshape(s.shape[0] // 8, 8, 128)


def _local_softmax(s):
    m = jnp.broadcast_to(jnp.max(jnp.max(_v3(s), axis=0), axis=0, keepdims=True), (8, 128))
    return jnp.exp2(_v3(s) - m[None]).reshape(s.shape), m


def _exchange(src, lane):
    grp = lane // 32
    odd = (grp & 1) == 1
    hi = grp >= 2
    live = [j for j in range(4) if src[j] is not None]

    def sel(m, a, b):
        if a is None:
            return b
        if b is None:
            return a
        return jnp.where(m, a, b)
    if len(live) == 2:
        out = [jnp.where(grp == (live[0] + i) % 4, src[live[0]], src[live[1]]) for i in range(4)]
    else:
        t = [sel(odd, src[(j + 1) % 4], src[j]) for j in range(4)]
        out = [sel(hi, t[(2 - i) % 4], t[(-i) % 4]) for i in range(4)]
    if len(live) < 4:
        res = []
        for i in range(4):
            dead = [(j + i) % 4 for j in range(4) if j not in live]
            m = grp == dead[0]
            for dd in dead[1:]:
                m = m | (grp == dd)
            res.append(jnp.where(m, jnp.zeros_like(out[i]), out[i]))
        out = res
    return out


def _qk(n, t=''):
    return [('qd' + t, n), ('qw' + t, n)]


def _pv(n, t=''):
    return [('pe' + t, n), ('pm' + t, n)]


def _weave(first, fills):
    prog = []
    for n in range(first, 16):
        prog += fills[n - first] + (_qk(n + 1) if n < 15 else []) + _pv(n)
    return prog


def _kernel(x_hbm, wqkv_hbm, wo_hbm, w1_hbm, w2_hbm, o_hbm,
            kwin, vwin, wvt, qbuf, obuf, xall, oall, wqk_ref, wv_ref, wo_ref, w1_ref, w2_ref, sems):
    step = pl.program_id(0)

    def xrows(i):
        return i * TQ if isinstance(i, int) else pl.multiple_of(i * TQ, TQ)

    def out_start(r, n, c0, c1):
        cols = slice(128 * c0, 128 * c1)
        pltpu.make_async_copy(oall.at[pl.ds(r, n), cols], o_hbm.at[0, pl.ds(r, n), cols], sems.at[12]).start()

    def shift():
        kwin[0:W // 2, :] = kwin[TQ // 2:TQ // 2 + W // 2, :]
        vwin[:, 0:W] = vwin[:, TQ:TQ + W]

    def stage_a(ops, tag, blk, r0, koff=W):
        R = 128
        h0 = r0 // 2
        lane_h = _lane(R // 2)
        st = {'k': {}, 'q': {}, 'kd': set(), 'qd': set()}

        def get_ln():
            if 'ln' not in st:
                st['ln'] = _ln(xall[pl.ds(xrows(blk) + r0, R), :].astype(f32))
            return st['ln']

        def get_xn():
            if 'xn' not in st:
                st['xn'] = get_ln().astype(bf)
            return st['xn']

        def finish(which, c0, c1, p):
            dst, roff = (kwin, koff // 2) if which == 'k' else (qbuf, 0)
            if which == 'q':
                p = p * QSCALE
            p = _pk(p.astype(bf))
            have = st[which]
            for c in range(c0, c1):
                have[c] = p[:, 128 * (c - c0):128 * (c - c0) + 128]
            for g in range(NG):
                a, b = _group_cols(g)
                if g not in st[which + 'd'] and a in have and b in have:
                    st[which + 'd'].add(g)
                    val = have[a] if a == b else jnp.where(lane_h >= (GW * g) % 128, have[a], have[b])
                    dst[roff + h0:roff + h0 + R // 2, 128 * g:128 * g + 128] = val

        def proj(which, c0, c1):
            off = D if which == 'k' else 0
            finish(which, c0, c1, jnp.dot(get_xn(), wqk_ref[:, off + 128 * c0:off + 128 * c1],
                                          preferred_element_type=f32))

        def projk(k):
            p = jnp.dot(get_ln()[:, 128 * k:128 * k + 128].astype(bf), wqk_ref[128 * k:128 * k + 128, :],
                        preferred_element_type=f32)
            if k:
                p = p + st['acc']
            st['acc'] = p
            if k == 4:
                finish('k', 0, 5, p[:, D:2 * D])
                finish('q', 0, 5, p[:, 0:D])

        def vproj(g0, g1):
            vt = lax.dot_general(_up(wvt[40 * g0:40 * g1, :]), get_xn(), NT, preferred_element_type=f32)
            row32 = lax.broadcasted_iota(jnp.int32, (32, R), 0)
            for h in range(4 * g0, 4 * g1):
                rr = 16 * ((DH * h) // 16) - 80 * g0
                jr = 0 if h % 4 == 3 else 31
                win = jnp.where(row32 == jr, 1.0, vt[rr:rr + 32, :])
                vwin[16 * h:16 * h + 16, koff + r0:koff + r0 + R] = _pk(win.astype(bf))
        ops['k' + tag] = lambda c0, c1: proj('k', c0, c1)
        ops['q' + tag] = lambda c0, c1: proj('q', c0, c1)
        ops['v' + tag] = vproj
        ops['ln' + tag] = get_ln
        ops['qk' + tag] = projk

    def stage_b(ops, first_block, tag=''):
        wb = -W if first_block else 0
        items = [(qb, g, min(qb, 2) if first_block else 2) for qb in range(2) for g in range(NG)]
        sts = [dict() for _ in items]
        parts = {0: {}, 1: {}}

        def qmask(n):
            qb, g, _ = items[n]
            st = sts[n]
            if 'M' not in st:
                lane16 = _lane(16)
                zero16 = jnp.zeros((16, 128), u32)
                nhm = [_not_head_lanes(4 * g + i, lane16) for i in range(4)]
                qs = [qbuf[64 * qb + 16 * j:64 * qb + 16 * j + 16, 128 * g:128 * g + 128] for j in range(4)]
                st['M'] = [[jnp.where(nhm[i], zero16, qs[j]) for j in range(4)] for i in range(4)]
            return st['M']

        def qd(n):
            qb, g, nprev = items[n]
            M = qmask(n)
            diag_first = lax.broadcasted_iota(jnp.int32, (32, 128), 0) > (_lane(32) % 32)
            hb = 64 * qb + wb // 2
            cs = slice(128 * g, 128 * g + 128)
            F = [[None] * 4 for _ in range(4)]
            L = [[None] * 4 for _ in range(4)]
            mD = []

            def cv(a):
                return _pk(a.astype(bf))
            for j in range(4):
                dt = _up(jnp.concatenate([M[(a - j) % 4][j] for a in range(4)], axis=0))
                klast = kwin[hb + 128:hb + 128 + 16 * (j + 1), cs]
                if nprev == 2:
                    kk = _up(jnp.concatenate([kwin[hb + 16 * j:hb + 64, cs], klast], axis=0))
                    sd = lax.dot_general(kk, dt, NT, preferred_element_type=f32)
                    e = jnp.where(diag_first, sd[0:32], sd[128:160])
                    sd = jnp.concatenate([e, sd[32:128]], axis=0)
                else:
                    sd = lax.dot_general(_up(klast), dt, NT, preferred_element_type=f32)
                    e = jnp.where(diag_first, NEG, sd[32 * j:32 * j + 32])
                    sd = jnp.concatenate([e, sd[0:32 * j]], axis=0) if j else e
                pd, m = _local_softmax(sd)
                mD.append(m)
                e = pd[0:32]
                rest = cv(pd[32:]) if pd.shape[0] > 32 else None
                k = 0
                if nprev == 2:
                    F[j][j] = cv(jnp.where(diag_first, e, 0.0))
                    L[j][j] = cv(jnp.where(diag_first, 0.0, e))
                    for b in range(j + 1, 4):
                        F[b][j] = rest[16 * k:16 * k + 16]
                        k += 1
                else:
                    L[j][j] = cv(e)
                for b in range(0, j):
                    L[b][j] = rest[16 * k:16 * k + 16]
                    k += 1
            sts[n].update(F=F, L=L, mD=mD)

        def qw(n):
            qb, g, nprev = items[n]
            if nprev == 0:
                return
            st = sts[n]
            M = qmask(n)
            kmid = _up(kwin[wb // 2 + 64 * qb + 64:wb // 2 + 64 * qb + 128, 128 * g:128 * g + 128])
            st['PW'], st['mW'] = [], []
            for i in range(4):
                wt = _up(jnp.concatenate([M[i][(a - i) % 4] for a in range(4)], axis=0))
                pw, m = _local_softmax(lax.dot_general(kmid, wt, NT, preferred_element_type=f32))
                st['PW'].append(pw.astype(bf))
                st['mW'].append(m)

        def pe(n):
            qb, g, nprev = items[n]
            st = sts[n]
            base = 128 * qb + wb
            lane16 = _lane(16)
            Fx = [_exchange(st['F'][b], lane16) for b in range(4)] if nprev == 2 else None
            Lx = [_exchange(st['L'][b], lane16) for b in range(4)]
            st['resE'] = []
            for i in range(4):
                rows = slice(16 * (4 * g + i), 16 * (4 * g + i) + 16)
                vl = vwin[rows, base + 256:base + 384]
                if nprev == 2:
                    p = jnp.concatenate([Fx[b][i] for b in range(4)] + [Lx[b][i] for b in range(4)], axis=0)
                    v = jnp.concatenate([vwin[rows, base:base + 128], vl], axis=1)
                else:
                    p = jnp.concatenate([Lx[b][i] for b in range(4)], axis=0)
                    v = vl
                st['resE'].append(jnp.dot(_up(v), _up(p), preferred_element_type=f32))

        def pm(n):
            qb, g, nprev = items[n]
            st = sts[n]
            base = 128 * qb + wb
            sub8 = lax.broadcasted_iota(jnp.int32, (8, 128), 0)
            if nprev >= 1:
                mE = _exchange(st['mD'], _lane(8))
            os_ = []
            for i in range(4):
                rows = slice(16 * (4 * g + i), 16 * (4 * g + i) + 16)
                res = st['resE'][i]
                if nprev >= 1:
                    resm = jnp.dot(_up(vwin[rows, base + 128:base + 256]), st['PW'][i],
                                   preferred_element_type=f32)
                    mx = jnp.maximum(mE[i], st['mW'][i])
                    ae = jnp.exp2(mE[i] - mx)
                    am = jnp.exp2(st['mW'][i] - mx)
                    res = (_v3(res) * ae[None] + _v3(resm) * am[None]).reshape(32, 128)
                jr = 0 if i == 3 else 31
                inv = 1.0 / res[jr:jr + 1, :]
                lo = (0, 0, 8, 8)[i]
                o = res[lo:lo + 24] * inv
                if i:
                    o = pltpu.roll(o, 128 - 32 * i, 1)
                os_.append(o)
            o0, o1, o2, o3 = os_
            parts[qb][g] = [o0[0:16], jnp.where(sub8 < 4, o0[16:24], o1[0:8]), o1[8:24],
                            o2[0:16], jnp.where(sub8 < 4, o2[16:24], o3[0:8]), o3[8:24]]
            st.clear()
            if len(parts[qb]) == NG:
                ot = jnp.concatenate([p for gg in range(NG) for p in parts[qb][gg]], axis=0)
                obuf[64 * qb:64 * qb + 64, :] = _pk(ot.astype(bf).T)
        ops.update({'qd' + tag: qd, 'qw' + tag: qw, 'pe' + tag: pe, 'pm' + tag: pm})

    def stage_c(ops, tag, blk, r0, R):
        st = {'f1': {}, 'f1b': {}, 'acc': {}}

        def c_wo():
            hres = xall[pl.ds(xrows(blk) + r0, R), :].astype(f32) + jnp.dot(
                _up(obuf[r0 // 2:(r0 + R) // 2, :]), wo_ref[...], preferred_element_type=f32)
            st['h'] = hres
            st['hn'] = _ln(hres).astype(bf)

        def c_f1(c0, c1):
            v = jnp.dot(st['hn'], w1_ref[:, 128 * c0:128 * c1], preferred_element_type=f32)
            v = jnp.maximum(v, 0.0)
            for c in range(c0, c1):
                st['f1'][c] = v[:, 128 * (c - c0):128 * (c - c0) + 128]

        def c_f2(c, k0, k1, ra=0, rb=R):
            key = (k0, k1, ra, rb)
            if key not in st['f1b']:
                st['f1b'][key] = jnp.concatenate(
                    [st['f1'][k][ra:rb] for k in range(k0, k1)], axis=1).astype(bf)
            v = jnp.dot(st['f1b'][key], w2_ref[128 * k0:128 * k1, 128 * c:128 * c + 128],
                        preferred_element_type=f32)
            if k0 == 0:
                acc = st['h'][ra:rb, 128 * c:128 * c + 128] + v
            else:
                acc = st['acc'][c][ra:rb] + v
            if k1 == 12:
                oall[pl.ds(xrows(blk) + r0 + ra, rb - ra), 128 * c:128 * c + 128] = acc.astype(bf)
            else:
                st['acc'][c] = acc
        ops['wo' + tag] = c_wo
        ops['f1' + tag] = c_f1
        ops['f2' + tag] = c_f2
        ops['out' + tag] = lambda c0, c1: out_start(xrows(blk) + r0, R, c0, c1)

    def run(ops, prog):
        for item in prog:
            ops[item[0]](*item[1:])

    @pl.when(step == 0)
    def _first():
        def cp_x(i, r0, r1):
            return pltpu.make_async_copy(x_hbm.at[0, r0:r1, :], xall.at[r0:r1, :], sems.at[i])
        cx0, cx1, cx2 = cp_x(0, 0, TQ), cp_x(1, TQ, 2 * TQ), cp_x(2, 2 * TQ, S)
        cp_qk = [pltpu.make_async_copy(wqkv_hbm.at[128 * k:128 * k + 128, 0:2 * D],
                                       wqk_ref.at[128 * k:128 * k + 128, :], sems.at[3 + k])
                 for k in range(5)]
        cp_v = pltpu.make_async_copy(wqkv_hbm.at[:, 2 * D:3 * D], wv_ref, sems.at[8])
        cp_o = pltpu.make_async_copy(wo_hbm, wo_ref, sems.at[9])
        cp_1 = pltpu.make_async_copy(w1_hbm, w1_ref, sems.at[10])
        cp_2 = pltpu.make_async_copy(w2_hbm, w2_ref, sems.at[11])
        for c in [cx0] + cp_qk + [cx1, cp_v, cp_o, cp_1, cp_2, cx2]:
            c.start()

        ops = {}
        stage_a(ops, 'L', 0, 0, 0)
        stage_a(ops, 'H', 0, 128, 0)
        stage_b(ops, True, 'a')
        stage_a(ops, '0', 1, 0)
        stage_a(ops, '1', 1, 128)
        stage_b(ops, False)
        stage_c(ops, '', 0, 0, TQ)

        def waits(*cps):
            for c in cps:
                c.wait()

        def xpose_wv():
            wvt[...] = _pk(wv_ref[...].T)
        ops.update(wait=waits, xpose=xpose_wv, shift=shift)

        def qa(*ns):
            return [o for n in ns for o in _qk(n, 'a')]

        def pa(*ns):
            return [o for n in ns for o in _pv(n, 'a')]
        prog = [('wait', cx0), ('lnL',), ('lnH',)]
        for k in range(5):
            prog += [('wait', cp_qk[k]), ('qkL', k), ('qkH', k)]
        prog += qa(*range(11))
        prog += [('wait', cx1, cp_v), ('xpose',)]
        prog += qa(11, 12) + [('k0', 0, 4)] + qa(13) + [('k0', 4, 5)] + qa(14) + [('vL', 0, 4), ('vL', 4, 8)]
        prog += qa(15) + pa(0) + [('vH', 0, 4)] + pa(1) + [('vH', 4, 8)] + pa(2, 3, 4) + [('q0', 0, 3)]
        prog += pa(5, 6) + [('q0', 3, 5)] + pa(7, 8) + [('v0', 0, 8)] + pa(9) + [('k1', 0, 4)] + pa(10)
        prog += [('k1', 4, 5)] + pa(11) + [('q1', 0, 1)] + pa(12) + _qk(0) + pa(13, 14, 15)
        prog += _qk(1) + _pv(0) + _qk(2) + _pv(1) + _qk(3) + _pv(2) + [('q1', 1, 5)]
        prog += [('wait', cp_o, cp_1, cp_2), ('wo',), ('v1', 0, 2), ('v1', 2, 4), ('v1', 4, 6), ('v1', 6, 8)]
        prog += _qk(4) + _pv(3) + _qk(5) + _pv(4)
        prog += _weave(5, [
            [('f1', 0, 2)], [('f1', 2, 4)], [('f1', 4, 6)], [('f1', 6, 8)],
            [('f2', 0, 0, 4), ('f1', 8, 10)], [('f1', 10, 12)], [('f2', 1, 0, 4), ('f2', 2, 0, 4)],
            [('f2', 3, 0, 4), ('f2', 4, 0, 4)], [('f2', 0, 4, 8), ('f2', 1, 4, 8), ('f2', 2, 4, 8)],
            [('f2', 3, 4, 8), ('f2', 4, 4, 8)], [('f2', 0, 8, 12), ('f2', 1, 8, 12), ('f2', 2, 8, 12)]])
        prog += [('f2', 3, 8, 12), ('shift',), ('f2', 4, 8, 12, 0, 128), ('f2', 4, 8, 12, 128, 256)]
        prog += [('out', 0, 5), ('wait', cx2)]
        run(ops, prog)

    @pl.when(jnp.logical_and(step > 0, step < NB - 1))
    def _mid():
        blk = step + 1
        ops = {'shift': shift}
        stage_c(ops, '', blk - 1, 0, TQ)
        stage_a(ops, '0', blk, 0)
        stage_a(ops, '1', blk, 128)
        stage_b(ops, False)
        prog = [('ln0',), ('wo',), ('k0', 0, 5), ('q0', 0, 5)] + _qk(0)
        prog += _weave(0, [
            [('v0', 0, 8)], [('q1', 0, 5)], [('k1', 0, 5)], [], [('f1', 0, 2)], [('v1', 0, 8)],
            [('f1', 2, 4)], [('f1', 4, 6)], [('f1', 6, 8)], [('f1', 8, 10)], [('f1', 10, 12)],
            [('f2', 0, 0, 6), ('f2', 1, 0, 6)], [('f2', 2, 0, 6)], [('f2', 3, 0, 6), ('f2', 4, 0, 6)],
            [('f2', 0, 6, 12)], [('f2', 1, 6, 12), ('f2', 2, 6, 12)]])
        prog += [('f2', 3, 6, 12), ('f2', 4, 6, 12, 0, 128), ('shift',), ('f2', 4, 6, 12, 128, 256)]
        prog += [('out', 0, 5)]
        run(ops, prog)

    @pl.when(step == NB - 1)
    def _last():
        ops = {}
        stage_c(ops, '0', NB - 1, 0, 128)
        stage_c(ops, '1', NB - 1, 128, 128)
        prog = [('wo0',), ('wo1',)]
        for t in '01':
            prog += [('f1' + t, 2 * c, 2 * c + 2) for c in range(6)]
        prog += [('f20', c, 0, 12) for c in range(5)] + [('out0', 0, 5)]
        prog += [('f21', c, 0, 12) for c in range(4)] + [('out1', 0, 4), ('f21', 4, 0, 12), ('out1', 4, 5)]
        run(ops, prog)
        pltpu.make_async_copy(oall, o_hbm.at[0], sems.at[12]).wait()


@jax.jit
def pallas_sequential_preLN__sliding_block__dense_activation_relu__prompt_kernel(
    A_x: jax.Array,
    A_wqkv: jax.Array,
    A_wo: jax.Array,
    B_x: jax.Array,
    B_w1: jax.Array,
    B_w2: jax.Array,
):
    del B_x
    hbm = pl.BlockSpec(memory_space=pl.ANY)
    return pl.pallas_call(
        _kernel,
        grid=(NB,),
        in_specs=[hbm] * 5,
        out_specs=hbm,
        out_shape=jax.ShapeDtypeStruct((1, S, D), bf),
        scratch_shapes=[
            pltpu.VMEM(((W + TQ) // 2, NG * 128), u32),
            pltpu.VMEM((H * 16, W + TQ), u32),
            pltpu.VMEM((D // 2, D), u32),
            pltpu.VMEM((TQ // 2, NG * 128), u32),
            pltpu.VMEM((TQ // 2, D), u32),
            pltpu.VMEM((S, D), bf),
            pltpu.VMEM((S, D), bf),
            pltpu.VMEM((D, 2 * D), bf),
            pltpu.VMEM((D, D), bf),
            pltpu.VMEM((D, D), bf),
            pltpu.VMEM((D, DFF), bf),
            pltpu.VMEM((DFF, D), bf),
            pltpu.SemaphoreType.DMA((13,)),
        ],
        compiler_params=pltpu.CompilerParams(
            dimension_semantics=("arbitrary",),
            vmem_limit_bytes=64 * 1024 * 1024,
            disable_bounds_checks=True,
            disable_semaphore_checks=True,
        ),
        name="fused",
    )(A_x, A_wqkv, A_wo, B_w1, B_w2)
```

```python
import math

import jax
import jax.numpy as jnp
from jax import lax
from jax.experimental import pallas as pl
from jax.experimental.pallas import tpu as pltpu

S, D, H, DH, W, DFF = 2048, 640, 32, 20, 256, 1536
TQ = 256
NB = S // TQ
NG = 8
GW = 4 * DH
EPS = 1e-5
LOG2E = math.log2(math.e)
QSCALE = DH ** -0.5 * LOG2E
NEG = -1e9 * LOG2E
bf = jnp.bfloat16
f32 = jnp.float32
u32 = jnp.uint32
NT = (((1,), (1,)), ((), ()))
NN = (((1,), (0,)), ((), ()))


def _pk(a):
    return pltpu.bitcast(a, u32)


def _up(a):
    return pltpu.bitcast(a, bf)


def _ln(x):
    m = jnp.mean(x, axis=-1, keepdims=True)
    xc = x - m
    v = jnp.mean(xc * xc, axis=-1, keepdims=True)
    return xc * lax.rsqrt(v + EPS)


def _lane(rows):
    return lax.broadcasted_iota(jnp.int32, (rows, 128), 1)


def _group_cols(g):
    lo = GW * g
    return lo // 128, (lo + GW - 1) // 128


def _not_head_lanes(h, lane):
    lo = (DH * h) % 128
    hi = lo + DH
    if hi <= 128:
        return (lane < lo) | (lane >= hi)
    return (lane < lo) & (lane >= hi - 128)


def _v3(s):
    return s.reshape(s.shape[0] // 8, 8, 128)


def _local_softmax(s):
    m = jnp.broadcast_to(jnp.max(jnp.max(_v3(s), axis=0), axis=0, keepdims=True), (8, 128))
    return jnp.exp2(_v3(s) - m[None]).reshape(s.shape), m


def _exchange(src, lane):
    grp = lane // 32
    odd = (grp & 1) == 1
    hi = grp >= 2
    live = [j for j in range(4) if src[j] is not None]

    def sel(m, a, b):
        if a is None:
            return b
        if b is None:
            return a
        return jnp.where(m, a, b)
    if len(live) == 2:
        out = [jnp.where(grp == (live[0] + i) % 4, src[live[0]], src[live[1]]) for i in range(4)]
    else:
        t = [sel(odd, src[(j + 1) % 4], src[j]) for j in range(4)]
        out = [sel(hi, t[(2 - i) % 4], t[(-i) % 4]) for i in range(4)]
    if len(live) < 4:
        res = []
        for i in range(4):
            dead = [(j + i) % 4 for j in range(4) if j not in live]
            m = grp == dead[0]
            for dd in dead[1:]:
                m = m | (grp == dd)
            res.append(jnp.where(m, jnp.zeros_like(out[i]), out[i]))
        out = res
    return out


def _qk(n, t=''):
    return [('qd' + t, n), ('qw' + t, n)]


def _pv(n, t=''):
    return [('pe' + t, n), ('pm' + t, n)]


def _weave(first, fills):
    prog = []
    for n in range(first, 16):
        prog += fills[n - first] + (_qk(n + 1) if n < 15 else []) + _pv(n)
    return prog


def _kernel(x_hbm, wqkv_hbm, wo_hbm, w1_hbm, w2_hbm, o_hbm,
            kwin, vwin, wvt, qbuf, obuf, xall, oall, wqk_ref, wv_ref, wo_ref, w1_ref, w2_ref, sems):
    step = pl.program_id(0)

    def xrows(i):
        return i * TQ if isinstance(i, int) else pl.multiple_of(i * TQ, TQ)

    def out_start(r, n, c0, c1):
        cols = slice(128 * c0, 128 * c1)
        pltpu.make_async_copy(oall.at[pl.ds(r, n), cols], o_hbm.at[0, pl.ds(r, n), cols], sems.at[12]).start()

    def shift():
        kwin[0:W // 2, :] = kwin[TQ // 2:TQ // 2 + W // 2, :]
        vwin[:, 0:W] = vwin[:, TQ:TQ + W]

    def stage_a(ops, tag, blk, r0, koff=W):
        R = 128
        h0 = r0 // 2
        lane_h = _lane(R // 2)
        st = {'k': {}, 'q': {}, 'kd': set(), 'qd': set()}

        def get_ln():
            if 'ln' not in st:
                st['ln'] = _ln(xall[pl.ds(xrows(blk) + r0, R), :].astype(f32))
            return st['ln']

        def get_xn():
            if 'xn' not in st:
                st['xn'] = get_ln().astype(bf)
            return st['xn']

        def finish(which, c0, c1, p):
            dst, roff = (kwin, koff // 2) if which == 'k' else (qbuf, 0)
            if which == 'q':
                p = p * QSCALE
            p = _pk(p.astype(bf))
            have = st[which]
            for c in range(c0, c1):
                have[c] = p[:, 128 * (c - c0):128 * (c - c0) + 128]
            for g in range(NG):
                a, b = _group_cols(g)
                if g not in st[which + 'd'] and a in have and b in have:
                    st[which + 'd'].add(g)
                    val = have[a] if a == b else jnp.where(lane_h >= (GW * g) % 128, have[a], have[b])
                    dst[roff + h0:roff + h0 + R // 2, 128 * g:128 * g + 128] = val

        def proj(which, c0, c1):
            off = D if which == 'k' else 0
            finish(which, c0, c1, jnp.dot(get_xn(), wqk_ref[:, off + 128 * c0:off + 128 * c1],
                                          preferred_element_type=f32))

        def projk(k):
            p = jnp.dot(get_ln()[:, 128 * k:128 * k + 128].astype(bf), wqk_ref[128 * k:128 * k + 128, :],
                        preferred_element_type=f32)
            if k:
                p = p + st['acc']
            st['acc'] = p
            if k == 4:
                finish('k', 0, 5, p[:, D:2 * D])
                finish('q', 0, 5, p[:, 0:D])

        def vproj(g0, g1):
            vt = lax.dot_general(_up(wvt[40 * g0:40 * g1, :]), get_xn(), NT, preferred_element_type=f32)
            row24 = lax.broadcasted_iota(jnp.int32, (24, R), 0)
            for h in range(4 * g0, 4 * g1):
                rr = 8 * ((DH * h) // 8) - 80 * g0
                jr = 0 if h % 2 else 23
                vwin[24 * h:24 * h + 24, koff + r0:koff + r0 + R] = jnp.where(row24 == jr, 1.0, vt[rr:rr + 24, :])
        ops['k' + tag] = lambda c0, c1: proj('k', c0, c1)
        ops['q' + tag] = lambda c0, c1: proj('q', c0, c1)
        ops['v' + tag] = vproj
        ops['ln' + tag] = get_ln
        ops['qk' + tag] = projk

    def stage_b(ops, first_block, tag=''):
        wb = -W if first_block else 0
        items = [(qb, g, min(qb, 2) if first_block else 2) for qb in range(2) for g in range(NG)]
        sts = [dict() for _ in items]
        parts = {0: {}, 1: {}}

        def qmask(n):
            qb, g, _ = items[n]
            st = sts[n]
            if 'M' not in st:
                lane16 = _lane(16)
                zero16 = jnp.zeros((16, 128), u32)
                nhm = [_not_head_lanes(4 * g + i, lane16) for i in range(4)]
                qs = [qbuf[64 * qb + 16 * j:64 * qb + 16 * j + 16, 128 * g:128 * g + 128] for j in range(4)]
                st['M'] = [[jnp.where(nhm[i], zero16, qs[j]) for j in range(4)] for i in range(4)]
            return st['M']

        def qd(n):
            qb, g, nprev = items[n]
            M = qmask(n)
            diag_first = lax.broadcasted_iota(jnp.int32, (32, 128), 0) > (_lane(32) % 32)
            hb = 64 * qb + wb // 2
            cs = slice(128 * g, 128 * g + 128)
            F = [[None] * 4 for _ in range(4)]
            L = [[None] * 4 for _ in range(4)]
            mD = []

            def cv(a):
                return _pk(a.astype(bf))
            for j in range(4):
                dt = _up(jnp.concatenate([M[(a - j) % 4][j] for a in range(4)], axis=0))
                klast = kwin[hb + 128:hb + 128 + 16 * (j + 1), cs]
                if nprev == 2:
                    kk = _up(jnp.concatenate([kwin[hb + 16 * j:hb + 64, cs], klast], axis=0))
                    sd = lax.dot_general(kk, dt, NT, preferred_element_type=f32)
                    e = jnp.where(diag_first, sd[0:32], sd[128:160])
                    sd = jnp.concatenate([e, sd[32:128]], axis=0)
                else:
                    sd = lax.dot_general(_up(klast), dt, NT, preferred_element_type=f32)
                    e = jnp.where(diag_first, NEG, sd[32 * j:32 * j + 32])
                    sd = jnp.concatenate([e, sd[0:32 * j]], axis=0) if j else e
                pd, m = _local_softmax(sd)
                mD.append(m)
                e = pd[0:32]
                rest = cv(pd[32:]) if pd.shape[0] > 32 else None
                k = 0
                if nprev == 2:
                    F[j][j] = cv(jnp.where(diag_first, e, 0.0))
                    L[j][j] = cv(jnp.where(diag_first, 0.0, e))
                    for b in range(j + 1, 4):
                        F[b][j] = rest[16 * k:16 * k + 16]
                        k += 1
                else:
                    L[j][j] = cv(e)
                for b in range(0, j):
                    L[b][j] = rest[16 * k:16 * k + 16]
                    k += 1
            sts[n].update(F=F, L=L, mD=mD)

        def qw(n):
            qb, g, nprev = items[n]
            if nprev == 0:
                return
            st = sts[n]
            M = qmask(n)
            kmid = _up(kwin[wb // 2 + 64 * qb + 64:wb // 2 + 64 * qb + 128, 128 * g:128 * g + 128])
            st['PW'], st['mW'] = [], []
            for i in range(4):
                wt = _up(jnp.concatenate([M[i][(a - i) % 4] for a in range(4)], axis=0))
                pw, m = _local_softmax(lax.dot_general(kmid, wt, NT, preferred_element_type=f32))
                st['PW'].append(pw.astype(bf))
                st['mW'].append(m)

        def vdot(g, i, k0, p):
            h = 4 * g + i
            return lax.dot_general(vwin[24 * h:24 * h + 24, k0:k0 + 128], p, NN, preferred_element_type=f32)

        def pe(n):
            qb, g, nprev = items[n]
            st = sts[n]
            lane16 = _lane(16)
            res = [None] * 4
            for which, off in (('F', 0), ('L', 256)):
                if which == 'F' and nprev < 2:
                    continue
                X = [_exchange(st[which][b], lane16) for b in range(4)]
                for i in range(4):
                    p = jnp.concatenate([X[b][i] for b in range(4)], axis=0)
                    r = vdot(g, i, 128 * qb + wb + off, _up(p))
                    res[i] = r if res[i] is None else res[i] + r
            st['resE'] = res

        def pm(n):
            qb, g, nprev = items[n]
            st = sts[n]
            sub8 = lax.broadcasted_iota(jnp.int32, (8, 128), 0)
            if nprev >= 1:
                resM = [vdot(g, i, 128 * qb + wb + 128, st['PW'][i]) for i in range(4)]
                mE = _exchange(st['mD'], _lane(8))
            os_ = []
            for i in range(4):
                res = st['resE'][i]
                if nprev >= 1:
                    mx = jnp.maximum(mE[i], st['mW'][i])
                    ae = jnp.exp2(mE[i] - mx)
                    am = jnp.exp2(st['mW'][i] - mx)
                    res = (_v3(res) * ae[None] + _v3(resM[i]) * am[None]).reshape(24, 128)
                jr = 0 if i % 2 else 23
                o = res * (1.0 / res[jr:jr + 1, :])
                if i:
                    o = pltpu.roll(o, 128 - 32 * i, 1)
                os_.append(o)
            o0, o1, o2, o3 = os_
            parts[qb][g] = [o0[0:16], jnp.where(sub8 < 4, o0[16:24], o1[0:8]), o1[8:24],
                            o2[0:16], jnp.where(sub8 < 4, o2[16:24], o3[0:8]), o3[8:24]]
            st.clear()
            if len(parts[qb]) == NG:
                ot = jnp.concatenate([p for gg in range(NG) for p in parts[qb][gg]], axis=0)
                obuf[64 * qb:64 * qb + 64, :] = _pk(ot.astype(bf).T)
        ops.update({'qd' + tag: qd, 'qw' + tag: qw, 'pe' + tag: pe, 'pm' + tag: pm})

    def stage_c(ops, tag, blk, r0, R):
        st = {'f1': {}, 'f1b': {}, 'acc': {}}

        def c_wo():
            hres = xall[pl.ds(xrows(blk) + r0, R), :].astype(f32) + jnp.dot(
                _up(obuf[r0 // 2:(r0 + R) // 2, :]), wo_ref[...], preferred_element_type=f32)
            st['h'] = hres
            st['hn'] = _ln(hres).astype(bf)

        def c_f1(c0, c1):
            v = jnp.dot(st['hn'], w1_ref[:, 128 * c0:128 * c1], preferred_element_type=f32)
            v = jnp.maximum(v, 0.0)
            for c in range(c0, c1):
                st['f1'][c] = v[:, 128 * (c - c0):128 * (c - c0) + 128]

        def c_f2(c, k0, k1, ra=0, rb=R):
            key = (k0, k1, ra, rb)
            if key not in st['f1b']:
                st['f1b'][key] = jnp.concatenate(
                    [st['f1'][k][ra:rb] for k in range(k0, k1)], axis=1).astype(bf)
            v = jnp.dot(st['f1b'][key], w2_ref[128 * k0:128 * k1, 128 * c:128 * c + 128],
                        preferred_element_type=f32)
            if k0 == 0:
                acc = st['h'][ra:rb, 128 * c:128 * c + 128] + v
            else:
                acc = st['acc'][c][ra:rb] + v
            if k1 == 12:
                oall[pl.ds(xrows(blk) + r0 + ra, rb - ra), 128 * c:128 * c + 128] = acc.astype(bf)
            else:
                st['acc'][c] = acc
        ops['wo' + tag] = c_wo
        ops['f1' + tag] = c_f1
        ops['f2' + tag] = c_f2
        ops['out' + tag] = lambda c0, c1: out_start(xrows(blk) + r0, R, c0, c1)

    def run(ops, prog):
        for item in prog:
            ops[item[0]](*item[1:])

    @pl.when(step == 0)
    def _first():
        def cp_x(i, r0, r1):
            return pltpu.make_async_copy(x_hbm.at[0, r0:r1, :], xall.at[r0:r1, :], sems.at[i])
        cx0, cx1, cx2 = cp_x(0, 0, TQ), cp_x(1, TQ, 2 * TQ), cp_x(2, 2 * TQ, S)
        cp_qk = [pltpu.make_async_copy(wqkv_hbm.at[128 * k:128 * k + 128, 0:2 * D],
                                       wqk_ref.at[128 * k:128 * k + 128, :], sems.at[3 + k])
                 for k in range(5)]
        cp_v = pltpu.make_async_copy(wqkv_hbm.at[:, 2 * D:3 * D], wv_ref, sems.at[8])
        cp_o = pltpu.make_async_copy(wo_hbm, wo_ref, sems.at[9])
        cp_1 = pltpu.make_async_copy(w1_hbm, w1_ref, sems.at[10])
        cp_2 = pltpu.make_async_copy(w2_hbm, w2_ref, sems.at[11])
        for c in [cx0] + cp_qk + [cx1, cp_v, cp_o, cp_1, cp_2, cx2]:
            c.start()

        ops = {}
        stage_a(ops, 'L', 0, 0, 0)
        stage_a(ops, 'H', 0, 128, 0)
        stage_b(ops, True, 'a')
        stage_a(ops, '0', 1, 0)
        stage_a(ops, '1', 1, 128)
        stage_b(ops, False)
        stage_c(ops, '', 0, 0, TQ)

        def waits(*cps):
            for c in cps:
                c.wait()

        def xpose_wv():
            wvt[...] = _pk(wv_ref[...].T)
        ops.update(wait=waits, xpose=xpose_wv, shift=shift)

        def qa(*ns):
            return [o for n in ns for o in _qk(n, 'a')]

        def pa(*ns):
            return [o for n in ns for o in _pv(n, 'a')]
        prog = [('wait', cx0), ('lnL',), ('lnH',)]
        for k in range(5):
            prog += [('wait', cp_qk[k]), ('qkL', k), ('qkH', k)]
        prog += qa(*range(11))
        prog += [('wait', cx1, cp_v), ('xpose',)]
        prog += qa(11, 12) + [('k0', 0, 2), ('k0', 2, 3)] + qa(13, 14, 15) + [('k0', 3, 5), ('vL', 0, 8)]
        prog += pa(0) + [('vH', 0, 8)] + pa(1, 2, 3, 4) + [('q0', 0, 2)] + pa(5, 6) + [('q0', 2, 5), ('v0', 0, 2)]
        prog += pa(7) + [('v0', 2, 4)] + pa(8, 9, 10, 11) + _qk(0) + _qk(1) + pa(12) + [('v0', 4, 6), ('v0', 6, 8)]
        prog += _pv(0) + [('k1', 0, 3)] + pa(13) + _pv(1) + pa(14) + [('k1', 3, 4), ('k1', 4, 5)] + _qk(2)
        prog += [('q1', 0, 1)] + pa(15) + _qk(3) + _pv(2) + _qk(4) + _pv(3) + [('q1', 1, 5)]
        prog += [('wait', cp_o, cp_1, cp_2), ('wo',), ('v1', 0, 4), ('v1', 4, 8)]
        prog += _qk(5) + _pv(4) + _qk(6) + _pv(5)
        prog += _weave(6, [
            [('f1', 0, 1), ('f1', 1, 2)], [('f1', 2, 4)], [('f1', 4, 6)], [('f1', 6, 8)], [('f1', 8, 10)],
            [('f1', 10, 11), ('f1', 11, 12), ('f2', 0, 0, 6)], [('f2', 2, 0, 6), ('f2', 1, 0, 6)],
            [('f2', 3, 0, 6)], [('f2', 4, 0, 6)], [('f2', 1, 6, 12), ('f2', 0, 6, 12), ('f2', 2, 6, 12)]])
        prog += [('f2', 4, 6, 12, 128, 256), ('f2', 3, 6, 12), ('f2', 4, 6, 12, 0, 128), ('shift',)]
        prog += [('out', 0, 5), ('wait', cx2)]
        run(ops, prog)

    @pl.when(jnp.logical_and(step > 0, step < NB - 1))
    def _mid():
        blk = step + 1
        ops = {'shift': shift}
        stage_c(ops, '', blk - 1, 0, TQ)
        stage_a(ops, '0', blk, 0)
        stage_a(ops, '1', blk, 128)
        stage_b(ops, False)
        prog = [('wo',), ('q0', 0, 5), ('k0', 0, 5)] + _qk(0)
        prog += _weave(0, [
            [('v0', 0, 8)], [('f1', 0, 2)], [('k1', 0, 2), ('k1', 2, 5)], [('f1', 2, 3), ('f1', 3, 4)],
            [('q1', 0, 2)], [('q1', 2, 5), ('v1', 0, 4)], [('v1', 4, 8), ('f2', 0, 0, 4)],
            [('f2', 1, 0, 4), ('f2', 2, 0, 4)], [('f1', 4, 6)], [('f1', 6, 8)],
            [('f2', 3, 0, 4), ('f2', 4, 0, 4), ('f2', 0, 4, 8)], [('f1', 10, 11), ('f1', 11, 12)],
            [('f1', 8, 10)], [('f2', 1, 4, 8)], [('f2', 2, 4, 8), ('f2', 1, 8, 12), ('f2', 2, 8, 12)],
            [('f2', 3, 4, 8), ('f2', 4, 4, 8), ('f2', 0, 8, 12)]])
        prog += [('f2', 3, 8, 12), ('f2', 4, 8, 12, 0, 128), ('shift',), ('f2', 4, 8, 12, 128, 256)]
        prog += [('out', 0, 5)]
        run(ops, prog)

    @pl.when(step == NB - 1)
    def _last():
        ops = {}
        stage_c(ops, '0', NB - 1, 0, 128)
        stage_c(ops, '1', NB - 1, 128, 128)
        prog = [('wo0',), ('wo1',)]
        for t in '01':
            prog += [('f1' + t, 2 * c, 2 * c + 2) for c in range(6)]
        prog += [('f20', c, 0, 12) for c in range(5)] + [('out0', 0, 5)]
        prog += [('f21', c, 0, 12) for c in range(4)] + [('out1', 0, 4), ('f21', 4, 0, 12), ('out1', 4, 5)]
        run(ops, prog)
        pltpu.make_async_copy(oall, o_hbm.at[0], sems.at[12]).wait()


@jax.jit
def pallas_sequential_preLN__sliding_block__dense_activation_relu__prompt_kernel(
    A_x: jax.Array,
    A_wqkv: jax.Array,
    A_wo: jax.Array,
    B_x: jax.Array,
    B_w1: jax.Array,
    B_w2: jax.Array,
):
    del B_x
    hbm = pl.BlockSpec(memory_space=pl.ANY)
    return pl.pallas_call(
        _kernel,
        grid=(NB,),
        in_specs=[hbm] * 5,
        out_specs=hbm,
        out_shape=jax.ShapeDtypeStruct((1, S, D), bf),
        scratch_shapes=[
            pltpu.VMEM(((W + TQ) // 2, NG * 128), u32),
            pltpu.VMEM((H * 24, W + TQ), f32),
            pltpu.VMEM((D // 2, D), u32),
            pltpu.VMEM((TQ // 2, NG * 128), u32),
            pltpu.VMEM((TQ // 2, D), u32),
            pltpu.VMEM((S, D), bf),
            pltpu.VMEM((S, D), bf),
            pltpu.VMEM((D, 2 * D), bf),
            pltpu.VMEM((D, D), bf),
            pltpu.VMEM((D, D), bf),
            pltpu.VMEM((D, DFF), bf),
            pltpu.VMEM((DFF, D), bf),
            pltpu.SemaphoreType.DMA((13,)),
        ],
        compiler_params=pltpu.CompilerParams(
            dimension_semantics=("arbitrary",),
            vmem_limit_bytes=64 * 1024 * 1024,
            disable_bounds_checks=True,
            disable_semaphore_checks=True,
        ),
        name="fused",
    )(A_x, A_wqkv, A_wo, B_w1, B_w2)
```

```python
import math

import jax
import jax.numpy as jnp
from jax import lax
from jax.experimental import pallas as pl
from jax.experimental.pallas import tpu as pltpu

S, D, H, DH, W, DFF = 2048, 640, 32, 20, 256, 1536
TQ = 256
NB = S // TQ
NG = 8
GW = 4 * DH
EPS = 1e-5
LOG2E = math.log2(math.e)
QSCALE = DH ** -0.5 * LOG2E
NEG = -1e9 * LOG2E
bf = jnp.bfloat16
f32 = jnp.float32
u32 = jnp.uint32
NT = (((1,), (1,)), ((), ()))
NN = (((1,), (0,)), ((), ()))


def _pk(a):
    return pltpu.bitcast(a, u32)


def _up(a):
    return pltpu.bitcast(a, bf)


def _ln(x):
    m = jnp.mean(x, axis=-1, keepdims=True)
    xc = x - m
    v = jnp.mean(xc * xc, axis=-1, keepdims=True)
    return xc * lax.rsqrt(v + EPS)


def _lane(rows):
    return lax.broadcasted_iota(jnp.int32, (rows, 128), 1)


def _group_cols(g):
    lo = GW * g
    return lo // 128, (lo + GW - 1) // 128


def _not_head_lanes(h, lane):
    lo = (DH * h) % 128
    hi = lo + DH
    if hi <= 128:
        return (lane < lo) | (lane >= hi)
    return (lane < lo) & (lane >= hi - 128)


def _v3(s):
    return s.reshape(s.shape[0] // 8, 8, 128)


def _local_softmax(s):
    m = jnp.broadcast_to(jnp.max(jnp.max(_v3(s), axis=0), axis=0, keepdims=True), (8, 128))
    return jnp.exp2(_v3(s) - m[None]).reshape(s.shape), m


def _exchange(src, lane):
    grp = lane // 32
    odd = (grp & 1) == 1
    hi = grp >= 2
    live = [j for j in range(4) if src[j] is not None]

    def sel(m, a, b):
        if a is None:
            return b
        if b is None:
            return a
        return jnp.where(m, a, b)
    if len(live) == 2:
        out = [jnp.where(grp == (live[0] + i) % 4, src[live[0]], src[live[1]]) for i in range(4)]
    else:
        t = [sel(odd, src[(j + 1) % 4], src[j]) for j in range(4)]
        out = [sel(hi, t[(2 - i) % 4], t[(-i) % 4]) for i in range(4)]
    if len(live) < 4:
        res = []
        for i in range(4):
            dead = [(j + i) % 4 for j in range(4) if j not in live]
            m = grp == dead[0]
            for dd in dead[1:]:
                m = m | (grp == dd)
            res.append(jnp.where(m, jnp.zeros_like(out[i]), out[i]))
        out = res
    return out


def _qk(n, t=''):
    return [('qd' + t, n), ('qw' + t, n)]


def _pv(n, t=''):
    return [('pe' + t, n), ('pm' + t, n)]


_FIRST_A = """
Qa11 Qa12 k0:0:2 k0:2:3 Qa13 Qa14 vL:0:8 Qa15 k0:3:4 k0:4:5 Pa0 vH:0:8 Pa1 Pa2 Pa3 q0:0:1 q0:1:2 Pa4
Pa5 Pa6 q0:2:5 v0:0:4 Pa7 Pa8 Pa9 Pa10 Pa11 v0:4:6 Q0 Q1 Pa12 k1:0:3 v0:6:8 P0 P1 Pa13 Pa14 k1:3:4
Q2 Pa15 Q3 k1:4:5 q1:0:1 P2 P3 q1:1:5
"""
_FIRST_B = """
wo:0:2 Q4 wo:2:3 wo:3:4 wo:4:5 v1:0:8 Q5 P4 Q6 P5 f1:0:1 f1:1:2 Q7 P6 f1:2:4 Q8 P7 f1:4:6 Q9 P8
f1:6:8 Q10 P9 f1:8:10 Q11 P10 f1:10:11 f1:11:12 f2:0:0:6 Q12 P11 f2:1:0:6 Q13 P12 f2:3:0:6 f2:2:0:6
Q14 P13 f2:4:0:6 Q15 f2:1:6:12 P14 f2:0:6:12 f2:2:6:12 P15 f2:4:6:12:128:256 f2:3:6:12 shift
f2:4:6:12:0:128
"""
_MID = """
wo:0:2 k0:0:1 wo:2:3 k1:0:1 q0:0:1 q0:1:2 q0:2:3 q0:3:4 q0:4:5 wo:3:5 k0:1:3 k0:3:4 k0:4:5 Q0 v0:0:8
Q1 P0 k1:1:2 k1:2:3 k1:3:5 Q2 P1 f1:0:1 f1:1:2 Q3 P2 q1:0:2 Q4 P3 f1:3:4 f1:2:3 Q5 P4 q1:2:4 q1:4:5
v1:0:1 v1:1:4 Q6 P5 v1:4:8 f2:0:0:4 Q7 P6 f2:2:0:4 f2:1:0:4 Q8 P7 f1:4:5 f1:5:6 Q9 P8 f1:6:7 f1:7:8
Q10 P9 f2:3:0:4 f2:4:0:4 Q11 P10 f2:1:4:8 Q12 P11 f2:0:4:8 f1:10:11 f1:11:12 Q13 P12 f1:8:9 f1:9:10
Q14 P13 f2:2:4:8 f2:2:8:12 f2:1:8:12 Q15 P14 f2:0:8:12 f2:4:4:8 f2:3:4:8 P15 f2:3:8:12
f2:4:8:12:0:128 shift f2:4:8:12:128:256
"""


def _parse(text):
    prog = []
    for tok in text.split():
        if tok[0] in 'QP':
            t = 'a' if tok[1] == 'a' else ''
            prog += (_qk if tok[0] == 'Q' else _pv)(int(tok[1 + len(t):]), t)
        else:
            name, *args = tok.split(':')
            prog.append((name, *map(int, args)))
    return prog


def _kernel(x_hbm, wqkv_hbm, wo_hbm, w1_hbm, w2_hbm, o_hbm,
            kwin, vwin, wvt, qbuf, obuf, xall, oall, wqk_ref, wv_ref, wo_ref, w1_ref, w2_ref, sems):
    step = pl.program_id(0)

    def xrows(i):
        return i * TQ if isinstance(i, int) else pl.multiple_of(i * TQ, TQ)

    def out_start(r, n, c0, c1):
        cols = slice(128 * c0, 128 * c1)
        pltpu.make_async_copy(oall.at[pl.ds(r, n), cols], o_hbm.at[0, pl.ds(r, n), cols], sems.at[12]).start()

    def shift():
        kwin[0:W // 2, :] = kwin[TQ // 2:TQ // 2 + W // 2, :]
        vwin[:, 0:W] = vwin[:, TQ:TQ + W]

    def stage_a(ops, tag, blk, r0, koff=W):
        R = 128
        h0 = r0 // 2
        lane_h = _lane(R // 2)
        st = {'k': {}, 'q': {}, 'kd': set(), 'qd': set()}

        def get_ln():
            if 'ln' not in st:
                st['ln'] = _ln(xall[pl.ds(xrows(blk) + r0, R), :].astype(f32))
            return st['ln']

        def get_xn():
            if 'xn' not in st:
                st['xn'] = get_ln().astype(bf)
            return st['xn']

        def finish(which, c0, c1, p):
            dst, roff = (kwin, koff // 2) if which == 'k' else (qbuf, 0)
            if which == 'q':
                p = p * QSCALE
            p = _pk(p.astype(bf))
            have = st[which]
            for c in range(c0, c1):
                have[c] = p[:, 128 * (c - c0):128 * (c - c0) + 128]
            for g in range(NG):
                a, b = _group_cols(g)
                if g not in st[which + 'd'] and a in have and b in have:
                    st[which + 'd'].add(g)
                    val = have[a] if a == b else jnp.where(lane_h >= (GW * g) % 128, have[a], have[b])
                    dst[roff + h0:roff + h0 + R // 2, 128 * g:128 * g + 128] = val

        def proj(which, c0, c1):
            off = D if which == 'k' else 0
            finish(which, c0, c1, jnp.dot(get_xn(), wqk_ref[:, off + 128 * c0:off + 128 * c1],
                                          preferred_element_type=f32))

        def projk(k):
            p = jnp.dot(get_ln()[:, 128 * k:128 * k + 128].astype(bf), wqk_ref[128 * k:128 * k + 128, :],
                        preferred_element_type=f32)
            if k:
                p = p + st['acc']
            st['acc'] = p
            if k == 4:
                finish('k', 0, 5, p[:, D:2 * D])
                finish('q', 0, 5, p[:, 0:D])

        def vproj(g0, g1):
            vt = lax.dot_general(_up(wvt[40 * g0:40 * g1, :]), get_xn(), NT, preferred_element_type=f32)
            row24 = lax.broadcasted_iota(jnp.int32, (24, R), 0)
            for h in range(4 * g0, 4 * g1):
                rr = 8 * ((DH * h) // 8) - 80 * g0
                jr = 0 if h % 2 else 23
                vwin[24 * h:24 * h + 24, koff + r0:koff + r0 + R] = jnp.where(row24 == jr, 1.0, vt[rr:rr + 24, :])
        ops['k' + tag] = lambda c0, c1: proj('k', c0, c1)
        ops['q' + tag] = lambda c0, c1: proj('q', c0, c1)
        ops['v' + tag] = vproj
        ops['ln' + tag] = get_ln
        ops['qk' + tag] = projk

    def stage_b(ops, first_block, tag=''):
        wb = -W if first_block else 0
        items = [(qb, g, min(qb, 2) if first_block else 2) for qb in range(2) for g in range(NG)]
        sts = [dict() for _ in items]
        parts = {0: {}, 1: {}}

        def qmask(n):
            qb, g, _ = items[n]
            st = sts[n]
            if 'M' not in st:
                lane16 = _lane(16)
                zero16 = jnp.zeros((16, 128), u32)
                nhm = [_not_head_lanes(4 * g + i, lane16) for i in range(4)]
                qs = [qbuf[64 * qb + 16 * j:64 * qb + 16 * j + 16, 128 * g:128 * g + 128] for j in range(4)]
                st['M'] = [[jnp.where(nhm[i], zero16, qs[j]) for j in range(4)] for i in range(4)]
            return st['M']

        def qd(n):
            qb, g, nprev = items[n]
            M = qmask(n)
            diag_first = lax.broadcasted_iota(jnp.int32, (32, 128), 0) > (_lane(32) % 32)
            hb = 64 * qb + wb // 2
            cs = slice(128 * g, 128 * g + 128)
            F = [[None] * 4 for _ in range(4)]
            L = [[None] * 4 for _ in range(4)]
            mD = []

            def cv(a):
                return _pk(a.astype(bf))
            for j in range(4):
                dt = _up(jnp.concatenate([M[(a - j) % 4][j] for a in range(4)], axis=0))
                klast = kwin[hb + 128:hb + 128 + 16 * (j + 1), cs]
                if nprev == 2:
                    kk = _up(jnp.concatenate([kwin[hb + 16 * j:hb + 64, cs], klast], axis=0))
                    sd = lax.dot_general(kk, dt, NT, preferred_element_type=f32)
                    e = jnp.where(diag_first, sd[0:32], sd[128:160])
                    sd = jnp.concatenate([e, sd[32:128]], axis=0)
                else:
                    sd = lax.dot_general(_up(klast), dt, NT, preferred_element_type=f32)
                    e = jnp.where(diag_first, NEG, sd[32 * j:32 * j + 32])
                    sd = jnp.concatenate([e, sd[0:32 * j]], axis=0) if j else e
                pd, m = _local_softmax(sd)
                mD.append(m)
                e = pd[0:32]
                rest = cv(pd[32:]) if pd.shape[0] > 32 else None
                k = 0
                if nprev == 2:
                    F[j][j] = cv(jnp.where(diag_first, e, 0.0))
                    L[j][j] = cv(jnp.where(diag_first, 0.0, e))
                    for b in range(j + 1, 4):
                        F[b][j] = rest[16 * k:16 * k + 16]
                        k += 1
                else:
                    L[j][j] = cv(e)
                for b in range(0, j):
                    L[b][j] = rest[16 * k:16 * k + 16]
                    k += 1
            sts[n].update(F=F, L=L, mD=mD)

        def qw(n):
            qb, g, nprev = items[n]
            if nprev == 0:
                return
            st = sts[n]
            M = qmask(n)
            kmid = _up(kwin[wb // 2 + 64 * qb + 64:wb // 2 + 64 * qb + 128, 128 * g:128 * g + 128])
            st['PW'], st['mW'] = [], []
            for i in range(4):
                wt = _up(jnp.concatenate([M[i][(a - i) % 4] for a in range(4)], axis=0))
                pw, m = _local_softmax(lax.dot_general(kmid, wt, NT, preferred_element_type=f32))
                st['PW'].append(pw.astype(bf))
                st['mW'].append(m)

        def vdot(g, i, k0, p):
            h = 4 * g + i
            return lax.dot_general(vwin[24 * h:24 * h + 24, k0:k0 + 128], p, NN, preferred_element_type=f32)

        def pe(n):
            qb, g, nprev = items[n]
            st = sts[n]
            lane16 = _lane(16)
            res = [None] * 4
            for which, off in (('F', 0), ('L', 256)):
                if which == 'F' and nprev < 2:
                    continue
                X = [_exchange(st[which][b], lane16) for b in range(4)]
                for i in range(4):
                    p = jnp.concatenate([X[b][i] for b in range(4)], axis=0)
                    r = vdot(g, i, 128 * qb + wb + off, _up(p))
                    res[i] = r if res[i] is None else res[i] + r
            st['resE'] = res

        def pm(n):
            qb, g, nprev = items[n]
            st = sts[n]
            sub8 = lax.broadcasted_iota(jnp.int32, (8, 128), 0)
            if nprev >= 1:
                resM = [vdot(g, i, 128 * qb + wb + 128, st['PW'][i]) for i in range(4)]
                mE = _exchange(st['mD'], _lane(8))
            os_ = []
            for i in range(4):
                res = st['resE'][i]
                if nprev >= 1:
                    mx = jnp.maximum(mE[i], st['mW'][i])
                    ae = jnp.exp2(mE[i] - mx)
                    am = jnp.exp2(st['mW'][i] - mx)
                    res = (_v3(res) * ae[None] + _v3(resM[i]) * am[None]).reshape(24, 128)
                jr = 0 if i % 2 else 23
                o = res * (1.0 / res[jr:jr + 1, :])
                if i:
                    o = pltpu.roll(o, 128 - 32 * i, 1)
                os_.append(o)
            o0, o1, o2, o3 = os_
            parts[qb][g] = [o0[0:16], jnp.where(sub8 < 4, o0[16:24], o1[0:8]), o1[8:24],
                            o2[0:16], jnp.where(sub8 < 4, o2[16:24], o3[0:8]), o3[8:24]]
            st.clear()
            if len(parts[qb]) == NG:
                ot = jnp.concatenate([p for gg in range(NG) for p in parts[qb][gg]], axis=0)
                obuf[64 * qb:64 * qb + 64, :] = _pk(ot.astype(bf).T)
        ops.update({'qd' + tag: qd, 'qw' + tag: qw, 'pe' + tag: pe, 'pm' + tag: pm})

    def stage_c(ops, tag, blk, r0, R):
        st = {'hp': [], 'f1': {}, 'f1b': {}, 'acc': {}}

        def c_wo(c0, c1):
            cols = slice(128 * c0, 128 * c1)
            st['hp'].append(xall[pl.ds(xrows(blk) + r0, R), cols].astype(f32) + jnp.dot(
                _up(obuf[r0 // 2:(r0 + R) // 2, :]), wo_ref[:, cols], preferred_element_type=f32))
            if c1 == 5:
                st['h'] = jnp.concatenate(st['hp'], axis=1) if c0 else st['hp'][0]
                st['hn'] = _ln(st['h']).astype(bf)

        def c_f1(c0, c1):
            v = jnp.dot(st['hn'], w1_ref[:, 128 * c0:128 * c1], preferred_element_type=f32)
            v = jnp.maximum(v, 0.0)
            for c in range(c0, c1):
                st['f1'][c] = v[:, 128 * (c - c0):128 * (c - c0) + 128]

        def c_f2(c, k0, k1, ra=0, rb=R):
            key = (k0, k1, ra, rb)
            if key not in st['f1b']:
                st['f1b'][key] = jnp.concatenate(
                    [st['f1'][k][ra:rb] for k in range(k0, k1)], axis=1).astype(bf)
            v = jnp.dot(st['f1b'][key], w2_ref[128 * k0:128 * k1, 128 * c:128 * c + 128],
                        preferred_element_type=f32)
            if k0 == 0:
                acc = st['h'][ra:rb, 128 * c:128 * c + 128] + v
            else:
                acc = st['acc'][c][ra:rb] + v
            if k1 == 12:
                oall[pl.ds(xrows(blk) + r0 + ra, rb - ra), 128 * c:128 * c + 128] = acc.astype(bf)
            else:
                st['acc'][c] = acc
        ops['wo' + tag] = c_wo
        ops['f1' + tag] = c_f1
        ops['f2' + tag] = c_f2
        ops['out' + tag] = lambda c0, c1: out_start(xrows(blk) + r0, R, c0, c1)

    def run(ops, prog):
        for item in prog:
            ops[item[0]](*item[1:])

    @pl.when(step == 0)
    def _first():
        def cp_x(i, r0, r1):
            return pltpu.make_async_copy(x_hbm.at[0, r0:r1, :], xall.at[r0:r1, :], sems.at[i])
        cx0, cx1, cx2 = cp_x(0, 0, TQ), cp_x(1, TQ, 2 * TQ), cp_x(2, 2 * TQ, S)
        cp_qk = [pltpu.make_async_copy(wqkv_hbm.at[128 * k:128 * k + 128, 0:2 * D],
                                       wqk_ref.at[128 * k:128 * k + 128, :], sems.at[3 + k])
                 for k in range(5)]
        cp_v = pltpu.make_async_copy(wqkv_hbm.at[:, 2 * D:3 * D], wv_ref, sems.at[8])
        cp_o = pltpu.make_async_copy(wo_hbm, wo_ref, sems.at[9])
        cp_1 = pltpu.make_async_copy(w1_hbm, w1_ref, sems.at[10])
        cp_2 = pltpu.make_async_copy(w2_hbm, w2_ref, sems.at[11])
        for c in [cx0] + cp_qk + [cx1, cp_v, cp_o, cp_1, cp_2, cx2]:
            c.start()

        ops = {}
        stage_a(ops, 'L', 0, 0, 0)
        stage_a(ops, 'H', 0, 128, 0)
        stage_b(ops, True, 'a')
        stage_a(ops, '0', 1, 0)
        stage_a(ops, '1', 1, 128)
        stage_b(ops, False)
        stage_c(ops, '', 0, 0, TQ)

        def waits(*cps):
            for c in cps:
                c.wait()

        def xpose_wv():
            wvt[...] = _pk(wv_ref[...].T)
        ops.update(wait=waits, xpose=xpose_wv, shift=shift)

        prog = [('wait', cx0), ('lnL',), ('lnH',)]
        for k in range(5):
            prog += [('wait', cp_qk[k]), ('qkL', k), ('qkH', k)]
        for n in range(11):
            prog += _qk(n, 'a')
        prog += [('wait', cx1, cp_v), ('xpose',)]
        prog += _parse(_FIRST_A) + [('wait', cp_o, cp_1, cp_2)] + _parse(_FIRST_B)
        prog += [('out', 0, 5), ('wait', cx2)]
        run(ops, prog)

    @pl.when(jnp.logical_and(step > 0, step < NB - 1))
    def _mid():
        blk = step + 1
        ops = {'shift': shift}
        stage_c(ops, '', blk - 1, 0, TQ)
        stage_a(ops, '0', blk, 0)
        stage_a(ops, '1', blk, 128)
        stage_b(ops, False)
        prog = _parse(_MID) + [('out', 0, 5)]
        run(ops, prog)

    @pl.when(step == NB - 1)
    def _last():
        ops = {}
        stage_c(ops, '0', NB - 1, 0, 128)
        stage_c(ops, '1', NB - 1, 128, 128)
        prog = [('wo0', 0, 5), ('wo1', 0, 5)]
        for t in '01':
            prog += [('f1' + t, 2 * c, 2 * c + 2) for c in range(6)]
        prog += [('f20', c, 0, 12) for c in range(5)] + [('out0', 0, 5)]
        prog += [('f21', c, 0, 12) for c in range(4)] + [('out1', 0, 4), ('f21', 4, 0, 12), ('out1', 4, 5)]
        run(ops, prog)
        pltpu.make_async_copy(oall, o_hbm.at[0], sems.at[12]).wait()


@jax.jit
def pallas_sequential_preLN__sliding_block__dense_activation_relu__prompt_kernel(
    A_x: jax.Array,
    A_wqkv: jax.Array,
    A_wo: jax.Array,
    B_x: jax.Array,
    B_w1: jax.Array,
    B_w2: jax.Array,
):
    del B_x
    hbm = pl.BlockSpec(memory_space=pl.ANY)
    return pl.pallas_call(
        _kernel,
        grid=(NB,),
        in_specs=[hbm] * 5,
        out_specs=hbm,
        out_shape=jax.ShapeDtypeStruct((1, S, D), bf),
        scratch_shapes=[
            pltpu.VMEM(((W + TQ) // 2, NG * 128), u32),
            pltpu.VMEM((H * 24, W + TQ), f32),
            pltpu.VMEM((D // 2, D), u32),
            pltpu.VMEM((TQ // 2, NG * 128), u32),
            pltpu.VMEM((TQ // 2, D), u32),
            pltpu.VMEM((S, D), bf),
            pltpu.VMEM((S, D), bf),
            pltpu.VMEM((D, 2 * D), bf),
            pltpu.VMEM((D, D), bf),
            pltpu.VMEM((D, D), bf),
            pltpu.VMEM((D, DFF), bf),
            pltpu.VMEM((DFF, D), bf),
            pltpu.SemaphoreType.DMA((13,)),
        ],
        compiler_params=pltpu.CompilerParams(
            dimension_semantics=("arbitrary",),
            vmem_limit_bytes=64 * 1024 * 1024,
            disable_bounds_checks=True,
            disable_semaphore_checks=True,
        ),
        name="fused",
    )(A_x, A_wqkv, A_wo, B_w1, B_w2)
```
